```python
import os as _os
_os.environ.setdefault("JAX_PLATFORMS", "cpu")
import jax
import jax.numpy as jnp

def _softmax(x, axis=-1):
    return jax.nn.softmax(x, axis=axis)
def _gelu(x):
    return jax.nn.gelu(x, approximate=True)
def _silu(x):
    return jax.nn.silu(x)
def _sigmoid(x):
    return jax.nn.sigmoid(x)
def _layernorm(x, axis=-1, eps=1e-5):
    m = jnp.mean(x, axis=axis, keepdims=True)
    v = jnp.var(x, axis=axis, keepdims=True)
    return (x - m) / jnp.sqrt(v + eps)
def _scatter_add(tgt, idx, src, axis=0):
    return tgt.at[idx].add(src)
def _segment_sum(src, seg, n):
    return jax.ops.segment_sum(src, seg, n)
class _Rng:
    def __init__(self, key):
        self._k = key
    def _next(self):
        self._k, sub = jax.random.split(self._k)
        return sub
    def normal(self, shape):
        return jax.random.normal(self._next(), shape, dtype=jnp.bfloat16)
    def randint(self, lo, hi, shape):
        return jax.random.randint(self._next(), shape, lo, hi, dtype=jnp.int32)
    def uniform(self, shape, lo=0.0, hi=1.0):
        return jax.random.uniform(self._next(), shape, jnp.bfloat16, lo, hi)
    def permutation(self, n):
        return jax.random.permutation(self._next(), n)


kernel_name = 'sequential_preLN__mha_block__moe_arch_mod__prompt'

def setup_inputs():
    _rng = _Rng(jax.random.key(int.from_bytes(__import__("os").urandom(4), "little")))
    _w = (lambda a: (lambda t: t.astype(jnp.bfloat16) if jnp.issubdtype(t.dtype, jnp.floating) else t)(jnp.asarray(a)))
    def _A_setup():
        B, S, D, H = 1, 2048, 512, 32
        return {
            "x": _w((lambda *s: _rng.normal(s) * 0.05)(B, S, D)),
            "wqkv": _w((lambda *s: _rng.normal(s) * 0.05)(D, 3 * D)),
            "wo": _w((lambda *s: _rng.normal(s) * 0.05)(D, D)),
        }
    _A_in = _A_setup()

    def _B_setup():
        B, S, D, F, C = 1, 2048, 512, 1792, 2
        return {
            "x": _w((lambda *s: _rng.normal(s) * 0.05)(B, S, D)),
            "w_r": _w((lambda *s: _rng.normal(s) * 0.05)(D)),
            "w_gate": _w((lambda *s: _rng.normal(s) * 0.05)(D, F)),
            "w_up": _w((lambda *s: _rng.normal(s) * 0.05)(D, F)),
            "w_down": _w((lambda *s: _rng.normal(s) * 0.05)(F, D)),
        }
    _B_in = _B_setup()

    return {
        "A_x": _A_in["x"],
        "A_wqkv": _A_in["wqkv"],
        "A_wo": _A_in["wo"],
        "B_x": _B_in["x"],
        "B_w_r": _B_in["w_r"],
        "B_w_gate": _B_in["w_gate"],
        "B_w_up": _B_in["w_up"],
        "B_w_down": _B_in["w_down"],
    }

def reference(A_x, A_wqkv, A_wo, B_x, B_w_r, B_w_gate, B_w_up, B_w_down):
    def _A_ref(x, wqkv, wo):
        B, S, D = x.shape
        H = 32
        Dh = D // H
        qkv = (lambda x, *d: x.transpose(*d))((x @ wqkv).reshape(B, S, 3, H, Dh), 2, 0, 3, 1, 4)
        q, k, v = qkv[0], qkv[1], qkv[2]
        scores = jnp.einsum("bhqd,bhkd->bhqk", q, k) * (Dh ** -0.5)
        p = _softmax(scores, axis=-1)
        o = jnp.einsum("bhqk,bhkd->bhqd", p, v)
        return (lambda x, *d: x.transpose(*d))(o, 0, 2, 1, 3).reshape(B, S, D) @ wo

    def _B_ref(x, w_r, w_gate, w_up, w_down):
        B, S, D = x.shape
        C = 2
        r = x @ w_r
        idx = jnp.argsort(-r, axis=-1)[:, :C]
        idx_e = jnp.repeat(idx.reshape(B, C, 1), D, axis=2)
        x_sel = jnp.take_along_axis(x, idx_e, axis=1)
        g = _silu(x_sel @ w_gate)
        u = x_sel @ w_up
        y = (g * u) @ w_down
        r_sel = _sigmoid(jnp.take_along_axis(r, idx, axis=1))
        y = y * r_sel.reshape(B, C, 1)
        b_off = (jnp.arange(B) * S).reshape(B, 1)
        flat_idx = (idx + b_off).reshape(B * C)
        zero = (x * 0.0).reshape(B * S, D)
        upd = _scatter_add(zero, flat_idx, y.reshape(B * C, D), axis=0)
        return x + upd.reshape(B, S, D)

    x = A_x
    h = x + _A_ref(_layernorm(x, axis=-1), A_wqkv, A_wo)
    h2 = h + _B_ref(_layernorm(h, axis=-1), B_w_r, B_w_gate, B_w_up, B_w_down)
    return h2
```

```python
import math

import jax
import jax.numpy as jnp
from jax import lax
import jax.experimental.pallas as pl
import jax.experimental.pallas.tpu as pltpu

f32, bf16, u32, i32 = jnp.float32, jnp.bfloat16, jnp.uint32, jnp.int32

H = 32
DH = 16
HG = 8
TQ = 512
CK = 128
LAG = 2
TB = 512
EPS = 1e-5
L_LO, L_HI = 2.0 ** -60, 2.0 ** 60


def _rb(x):
    return x.astype(bf16).astype(f32)


def _layernorm(x):
    d = x.shape[-1]
    mean = jnp.sum(x, axis=-1, keepdims=True) * (1.0 / d)
    xc = x - mean
    var = jnp.sum(xc * xc, axis=-1, keepdims=True) * (1.0 / d)
    den = _rb(jnp.sqrt(_rb(_rb(var) + EPS)))
    return _rb(x - _rb(mean)) * (1.0 / den)


def _pack(x):
    return pltpu.bitcast(x.astype(bf16), u32)


def _unpack(x):
    return pltpu.bitcast(x, bf16)


def _kernel(x_ref, wqkv_ref, wr_ref, wo_hbm, wg_hbm, wu_hbm, wd_hbm, o_ref,
            kp_ref, qp_ref, vp_ref, op_ref, l_ref, h_ref, r_ref, wt_ref,
            wo_ref, wg_ref, wu_ref, wd_ref, sems):
    S, D = x_ref.shape
    NQ = S // TQ
    NC = S // CK
    NG = H // HG

    copies = [pltpu.make_async_copy(src, dst, sems.at[i]) for i, (src, dst) in enumerate(
        ((wo_hbm, wo_ref), (wg_hbm, wg_ref), (wu_hbm, wu_ref), (wd_hbm, wd_ref)))]
    for cp in copies:
        cp.start()

    wt_ref[0:D, :] = wqkv_ref[:, 0:D].astype(f32).T.astype(bf16)
    wt_ref[D:2 * D, :] = wqkv_ref[:, 2 * D:3 * D].astype(f32).T.astype(bf16)
    qscale = (DH ** -0.5) * math.log2(math.e)
    for b in range(S // TB):
        xn = _layernorm(x_ref[b * TB:(b + 1) * TB, :].astype(f32)).astype(bf16)
        k = jnp.dot(xn, wqkv_ref[:, D:2 * D], preferred_element_type=f32)
        for g in range(NG):
            kp_ref[g, b * TB // 2:(b + 1) * TB // 2, :] = _pack(k[:, g * 128:(g + 1) * 128])
        qv = lax.dot_general(wt_ref[...], xn, (((1,), (1,)), ((), ())),
                             preferred_element_type=f32)
        qp_ref[:, b * TB:(b + 1) * TB] = _pack(_rb(qv[0:D]) * qscale)
        vp_ref[:, b * TB:(b + 1) * TB] = _pack(qv[D:2 * D])

    def q_weights(h8, j, cols):
        qrow = qp_ref[pl.ds(h8, 8), cols]
        z = jnp.zeros_like(qrow)
        return _unpack(jnp.concatenate([qrow if b == j else z for b in range(HG)], axis=0))

    def k_chunk(g, c):
        base = c * (CK // 2)
        return _unpack(jnp.concatenate(
            [kp_ref[g, base + (7 - b) * 8:base + (8 - b) * 8, :] for b in range(8)], axis=0))

    def unreverse(p):
        return jnp.concatenate([p[(7 - b) * 16:(8 - b) * 16, :] for b in range(8)], axis=0)

    def fast_group(i, carry):
        qb = i // NG
        g = i % NG
        cols = pl.ds(pl.multiple_of(qb * TQ, TQ), TQ)
        h8s = [pl.multiple_of((g * HG + j) * 8, 8) for j in range(HG)]
        pend = []
        l8 = [None] * HG
        acc = [None] * HG

        def pv(j, c, p):
            vt = _unpack(vp_ref[pl.ds(h8s[j], 8), c * CK:(c + 1) * CK])
            d = jnp.dot(vt, p, preferred_element_type=f32)
            acc[j] = d if acc[j] is None else acc[j] + d
            if c == NC - 1:
                l = jnp.sum(l8[j], axis=0, keepdims=True)
                l_ref[pl.ds(g * HG + j, 1), cols] = l
                op_ref[pl.ds(h8s[j], 8), cols] = _pack(acc[j] * (1.0 / l))

        for j in range(HG):
            w = q_weights(h8s[j], j, cols)
            for c in range(NC):
                s = jnp.dot(k_chunk(g, c), w, preferred_element_type=f32)
                p = jnp.exp2(s)
                cl = jnp.sum(p.reshape(CK // 8, 8, TQ), axis=0)
                l8[j] = cl if l8[j] is None else l8[j] + cl
                pend.append((j, c, unreverse(p).astype(bf16)))
                if len(pend) > LAG:
                    pv(*pend.pop(0))
        for item in pend:
            pv(*item)
        return carry

    lax.fori_loop(0, NQ * NG, fast_group, 0)

    l_all = l_ref[...]
    safe = jnp.logical_and(jnp.min(l_all) >= L_LO, jnp.max(l_all) <= L_HI)

    @pl.when(jnp.logical_not(safe))
    def _():
        def unit(u, carry):
            qb = u // H
            h = u % H
            g = h // HG
            j = h % HG
            cols = pl.ds(pl.multiple_of(qb * TQ, TQ), TQ)
            h8 = pl.multiple_of(h * 8, 8)
            qrow = qp_ref[pl.ds(h8, 8), cols]
            z = jnp.zeros_like(qrow)
            w = _unpack(jnp.concatenate(
                [jnp.where(j == b, qrow, z) for b in range(HG)], axis=0))

            def scores(c):
                rows = pl.ds(pl.multiple_of(c * (CK // 2), CK // 2), CK // 2)
                return jnp.dot(_unpack(kp_ref[g, rows, :]), w, preferred_element_type=f32)

            def max_body(c, m):
                return jnp.maximum(m, jnp.max(scores(c), axis=0, keepdims=True))

            m = lax.fori_loop(0, NC, max_body, jnp.full((1, TQ), -jnp.inf, f32))

            def sum_body(c, la):
                l, a = la
                p = jnp.exp2(scores(c) - m)
                vt = _unpack(vp_ref[pl.ds(h8, 8), pl.ds(pl.multiple_of(c * CK, CK), CK)])
                a = a + jnp.dot(vt, p.astype(bf16), preferred_element_type=f32)
                return l + jnp.sum(p, axis=0, keepdims=True), a

            l, a = lax.fori_loop(0, NC, sum_body,
                                 (jnp.zeros((1, TQ), f32), jnp.zeros((DH, TQ), f32)))
            op_ref[pl.ds(h8, 8), cols] = _pack(a * (1.0 / l))
            return carry

        lax.fori_loop(0, NQ * H, unit, 0)

    copies[0].wait()
    wr = jnp.broadcast_to(wr_ref[...], (16, D))
    for b in range(S // TB):
        rows = slice(b * TB, (b + 1) * TB)
        ot = _unpack(op_ref[:, rows])
        attn = lax.dot_general(ot, wo_ref[...], (((0,), (0,)), ((), ())),
                               preferred_element_type=f32)
        h = _rb(x_ref[rows, :].astype(f32) + _rb(attn))
        hn = _layernorm(h).astype(bf16)
        h_ref[rows, :] = h
        o_ref[rows, :] = (h + hn.astype(f32)).astype(bf16)
        r = lax.dot_general(wr, hn, (((1,), (1,)), ((), ())), preferred_element_type=f32)
        r_ref[b:b + 1, :] = _rb(r[0:1, :])

    r = r_ref[...]
    tok = (lax.broadcasted_iota(i32, r.shape, 0) * TB + lax.broadcasted_iota(i32, r.shape, 1))
    m1 = jnp.max(r)
    i1 = jnp.min(jnp.where(r == m1, tok, S - 1))
    r2 = jnp.where(tok == i1, -jnp.inf, r)
    m2 = jnp.max(r2)
    i2 = jnp.min(jnp.where(jnp.logical_and(r2 == m2, tok != i1), tok, S - 1))

    row16 = lax.broadcasted_iota(i32, (16, D), 0)
    h1 = h_ref[pl.ds(i1, 1), :]
    h2 = h_ref[pl.ds(i2, 1), :]
    hsel = jnp.where(row16 == 0, h1, h2)
    xsel = _layernorm(hsel).astype(bf16)
    copies[1].wait()
    copies[2].wait()
    copies[3].wait()
    gpre = _rb(jnp.dot(xsel, wg_ref[...], preferred_element_type=f32))
    gate = _rb(gpre * jax.nn.sigmoid(gpre))
    up = _rb(jnp.dot(xsel, wu_ref[...], preferred_element_type=f32))
    y = _rb(jnp.dot((gate * up).astype(bf16), wd_ref[...], preferred_element_type=f32))
    rsel = _rb(jax.nn.sigmoid(jnp.where(row16 == 0, m1, m2)))
    y = _rb(y * rsel)
    y1 = y[0:1, :]
    y2 = y[1:2, :]
    for idx in (i1, i2):
        base = pl.multiple_of((idx // 16) * 16, 16)
        hg = h_ref[pl.ds(base, 16), :]
        hng = _rb(_layernorm(hg))
        t = row16 + base
        upd = jnp.where(t == i1, y1, jnp.where(t == i2, y2, 0.0))
        o_ref[pl.ds(base, 16), :] = (hg + _rb(hng + upd)).astype(bf16)


@jax.jit
def pallas_sequential_preLN__mha_block__moe_arch_mod__prompt_kernel(
    A_x: jax.Array,
    A_wqkv: jax.Array,
    A_wo: jax.Array,
    B_x: jax.Array,
    B_w_r: jax.Array,
    B_w_gate: jax.Array,
    B_w_up: jax.Array,
    B_w_down: jax.Array,
):
    B, S, D = A_x.shape
    F = B_w_gate.shape[1]
    assert B == 1 and D == H * DH and S % TQ == 0 and S % TB == 0
    vmem = pl.BlockSpec(memory_space=pltpu.VMEM)
    hbm = pl.BlockSpec(memory_space=pl.ANY)
    out = pl.pallas_call(
        _kernel,
        out_shape=jax.ShapeDtypeStruct((S, D), A_x.dtype),
        in_specs=[vmem, vmem, vmem, hbm, hbm, hbm, hbm],
        out_specs=vmem,
        scratch_shapes=[
            pltpu.VMEM((H // HG, S // 2, 128), u32),
            pltpu.VMEM((D // 2, S), u32),
            pltpu.VMEM((D // 2, S), u32),
            pltpu.VMEM((D // 2, S), u32),
            pltpu.VMEM((H, S), f32),
            pltpu.VMEM((S, D), f32),
            pltpu.VMEM((S // TB, TB), f32),
            pltpu.VMEM((2 * D, D), bf16),
            pltpu.VMEM((D, D), bf16),
            pltpu.VMEM((D, F), bf16),
            pltpu.VMEM((D, F), bf16),
            pltpu.VMEM((F, D), bf16),
            pltpu.SemaphoreType.DMA((4,)),
        ],
        compiler_params=pltpu.CompilerParams(vmem_limit_bytes=100 * 1024 * 1024),
    )(A_x.reshape(S, D), A_wqkv, B_w_r.reshape(1, D), A_wo, B_w_gate, B_w_up, B_w_down)
    return out.reshape(B, S, D)
```

```python
import math

import jax
import jax.numpy as jnp
from jax import lax
import jax.experimental.pallas as pl
import jax.experimental.pallas.tpu as pltpu

f32, bf16, u32, i32 = jnp.float32, jnp.bfloat16, jnp.uint32, jnp.int32

H = 32
DH = 16
HG = 8
TQ = 512
CK = 128
LAG = 2
RING = 4
TP = 256
TB = 512
EPS = 1e-5
L_LO, L_HI = 2.0 ** -60, 2.0 ** 60


def _rb(x):
    return x.astype(bf16).astype(f32)


def _layernorm(x):
    d = x.shape[-1]
    mean = jnp.sum(x, axis=-1, keepdims=True) * (1.0 / d)
    xc = x - mean
    var = jnp.sum(xc * xc, axis=-1, keepdims=True) * (1.0 / d)
    den = _rb(jnp.sqrt(_rb(_rb(var) + EPS)))
    return _rb(x - _rb(mean)) * (1.0 / den)


def _pack(x):
    return pltpu.bitcast(x.astype(bf16), u32)


def _unpack(x):
    return pltpu.bitcast(x, bf16)


def _kernel(x_ref, wqkv_ref, wr_ref, wo_hbm, wg_hbm, wu_hbm, wd_hbm, o_ref,
            kp_ref, kv_ref, kb_ref, qp_ref, vp_ref, op_ref, l_ref, h_ref, r_ref, wt_ref,
            wo_ref, wg_ref, wu_ref, wd_ref, sems, *stage):
    pt_refs = stage[:RING]
    qs_refs = stage[RING:]
    S, D = x_ref.shape
    NQ = S // TQ
    NC = S // CK
    NG = H // HG

    copies = [pltpu.make_async_copy(src, dst, sems.at[i]) for i, (src, dst) in enumerate(
        ((wo_hbm, wo_ref), (wg_hbm, wg_ref), (wu_hbm, wu_ref), (wd_hbm, wd_ref)))]
    for cp in copies:
        cp.start()

    xv = jnp.concatenate([x_ref[c * CK:c * CK + 16, :] for c in range(NC)], axis=0)
    kv = jnp.dot(_layernorm(xv.astype(f32)).astype(bf16), wqkv_ref[:, D:2 * D],
                 preferred_element_type=f32)
    for g in range(NG):
        kv_ref[g] = _pack(kv[:, g * 128:(g + 1) * 128])
    wt_ref[0:D, :] = wqkv_ref[:, 0:D].astype(f32).T.astype(bf16)
    wt_ref[D:2 * D, :] = wqkv_ref[:, 2 * D:3 * D].astype(f32).T.astype(bf16)
    qscale = (DH ** -0.5) * math.log2(math.e)

    NP = S // TP

    def ln_block(b):
        rows = pl.ds(pl.multiple_of(b * TP, TP), TP)
        return _layernorm(x_ref[rows, :].astype(f32)).astype(bf16)

    def proj(b, carry):
        rows = pl.ds(pl.multiple_of(b * TP, TP), TP)
        xn = ln_block(b)
        kks = {}
        for cc in range(TP // CK):
            c = b * (TP // CK) + cc
            for g in range(NG):
                kks[cc, g] = _unpack(kv_ref[g, pl.ds(pl.multiple_of(c * 8, 8), 8), :]).astype(f32)
        for jd in range(128):
            for cc in range(TP // CK):
                c = b * (TP // CK) + cc
                for g in range(NG):
                    kb_ref[g * 128 + jd, pl.ds(pl.multiple_of(c * 16, 16), 16), :] = (
                        jnp.broadcast_to(kks[cc, g][:, jd:jd + 1], (16, 128)))
        k = jnp.dot(xn, wqkv_ref[:, D:2 * D], preferred_element_type=f32)
        for g in range(NG):
            kp_ref[g, pl.ds(pl.multiple_of(b * (TP // 2), TP // 2), TP // 2), :] = (
                _pack(k[:, g * 128:(g + 1) * 128]))
        qv = lax.dot_general(wt_ref[...], xn, (((1,), (1,)), ((), ())),
                             preferred_element_type=f32)
        qp_ref[:, rows] = _pack(_rb(qv[0:D]) * qscale)
        vp_ref[:, rows] = _pack(qv[D:2 * D])
        return carry

    lax.fori_loop(0, NP, proj, 0)

    def fast_group(i, carry):
        qb = i // NG
        g = i % NG
        cols = pl.ds(pl.multiple_of(qb * TQ, TQ), TQ)
        hs = [g * HG + j for j in range(HG)]
        h8s = [pl.multiple_of(h * 8, 8) for h in hs]
        z1 = lax.shift_right_logical(i, 20)
        zz = pl.multiple_of(z1 * 8, 8)
        never = lax.broadcasted_iota(i32, (16, 128), 0) < z1
        pend = []
        l8 = [None] * HG
        acc = [None] * HG

        def pv(j, c, slot):
            vt = _unpack(vp_ref[pl.ds(h8s[j], 8), c * CK:(c + 1) * CK])
            d = jnp.dot(vt, _unpack(pt_refs[slot][pl.ds(zz, CK // 2), :]),
                        preferred_element_type=f32)
            acc[j] = d if acc[j] is None else acc[j] + d
            if c == NC - 1:
                l = jnp.sum(l8[j], axis=0, keepdims=True)
                l_ref[pl.ds(hs[j], 1), cols] = l
                op_ref[pl.ds(h8s[j], 8), cols] = _pack(acc[j] * (1.0 / l))

        def vpu_block(j, c, slot):
            tiles = []
            for t in range(TQ // 128):
                a = None
                for d in range(DH):
                    kb = kb_ref[hs[j] * DH + d, c * 16:(c + 1) * 16, :]
                    qd = qs_refs[j][z1 + d, :, t * 128:(t + 1) * 128]
                    pr = kb * jnp.concatenate([qd, qd], axis=0)
                    if a is None:
                        a = pr if t == 0 else jnp.where(never, tiles[t - 1], pr)
                    else:
                        a = a + pr
                tiles.append(a)
            p = jnp.exp2(jnp.concatenate(tiles, axis=1))
            l8[j] = l8[j] + (p[0:8] + p[8:16])
            pt_refs[slot][0:8, :] = _pack(p)

        for j in range(HG):
            qrow = qp_ref[pl.ds(h8s[j], 8), cols]
            z = jnp.zeros_like(qrow)
            w = _unpack(jnp.concatenate([qrow if b == j else z for b in range(HG)], axis=0))
            qf = _unpack(qrow).astype(f32)
            for d in range(DH):
                qs_refs[j][d] = jnp.broadcast_to(qf[d:d + 1, :], (8, TQ))
            for c in range(NC):
                slot = (j * NC + c) % RING
                base = c * (CK // 2)
                kc = _unpack(jnp.concatenate(
                    [kp_ref[g, base + b * 8:base + (b + 1) * 8, :] for b in range(7, 0, -1)],
                    axis=0))
                s = jnp.dot(kc, w, preferred_element_type=f32)
                p = jnp.exp2(s)
                cl = jnp.sum(p.reshape(14, 8, TQ), axis=0)
                l8[j] = cl if l8[j] is None else l8[j] + cl
                for b in range(7):
                    pt_refs[slot][(7 - b) * 8:(8 - b) * 8, :] = _pack(p[b * 16:(b + 1) * 16, :])
                pend.append((j, c, slot))
                if len(pend) > LAG:
                    pv(*pend.pop(0))
                vpu_block(j, c, slot)
        for item in pend:
            pv(*item)
        return carry

    lax.fori_loop(0, NQ * NG, fast_group, 0)

    l_all = l_ref[...]
    safe = jnp.logical_and(jnp.min(l_all) >= L_LO, jnp.max(l_all) <= L_HI)

    @pl.when(jnp.logical_not(safe))
    def _():
        def unit(u, carry):
            qb = u // H
            h = u % H
            g = h // HG
            j = h % HG
            cols = pl.ds(pl.multiple_of(qb * TQ, TQ), TQ)
            h8 = pl.multiple_of(h * 8, 8)
            qrow = qp_ref[pl.ds(h8, 8), cols]
            z = jnp.zeros_like(qrow)
            w = _unpack(jnp.concatenate(
                [jnp.where(j == b, qrow, z) for b in range(HG)], axis=0))

            def scores(c):
                rows = pl.ds(pl.multiple_of(c * (CK // 2), CK // 2), CK // 2)
                return jnp.dot(_unpack(kp_ref[g, rows, :]), w, preferred_element_type=f32)

            def max_body(c, m):
                return jnp.maximum(m, jnp.max(scores(c), axis=0, keepdims=True))

            m = lax.fori_loop(0, NC, max_body, jnp.full((1, TQ), -jnp.inf, f32))

            def sum_body(c, la):
                l, a = la
                p = jnp.exp2(scores(c) - m)
                vt = _unpack(vp_ref[pl.ds(h8, 8), pl.ds(pl.multiple_of(c * CK, CK), CK)])
                a = a + jnp.dot(vt, p.astype(bf16), preferred_element_type=f32)
                return l + jnp.sum(p, axis=0, keepdims=True), a

            l, a = lax.fori_loop(0, NC, sum_body,
                                 (jnp.zeros((1, TQ), f32), jnp.zeros((DH, TQ), f32)))
            op_ref[pl.ds(h8, 8), cols] = _pack(a * (1.0 / l))
            return carry

        lax.fori_loop(0, NQ * H, unit, 0)

    copies[0].wait()
    wr = wr_ref[...]
    for b in range(S // TB):
        rows = slice(b * TB, (b + 1) * TB)
        ot = _unpack(op_ref[:, rows])
        attn = lax.dot_general(ot, wo_ref[...], (((0,), (0,)), ((), ())),
                               preferred_element_type=f32)
        h = _rb(x_ref[rows, :].astype(f32) + _rb(attn))
        hn = _layernorm(h).astype(bf16)
        h_ref[rows, :] = h
        o_ref[rows, :] = (h + hn.astype(f32)).astype(bf16)
        r = lax.dot_general(wr, hn, (((1,), (1,)), ((), ())), preferred_element_type=f32)
        r_ref[b:b + 1, :] = _rb(r[0:1, :])

    r = r_ref[0:S // TB, :]
    tok = (lax.broadcasted_iota(i32, r.shape, 0) * TB + lax.broadcasted_iota(i32, r.shape, 1))
    m1 = jnp.max(r)
    i1 = jnp.min(jnp.where(r == m1, tok, S - 1))
    r2 = jnp.where(tok == i1, -jnp.inf, r)
    m2 = jnp.max(r2)
    i2 = jnp.min(jnp.where(jnp.logical_and(r2 == m2, tok != i1), tok, S - 1))

    row16 = lax.broadcasted_iota(i32, (16, D), 0)
    h1 = h_ref[pl.ds(i1, 1), :]
    h2 = h_ref[pl.ds(i2, 1), :]
    hsel = jnp.where(row16 == 0, h1, h2)
    xsel = _layernorm(hsel).astype(bf16)
    copies[1].wait()
    copies[2].wait()
    copies[3].wait()
    gpre = _rb(jnp.dot(xsel, wg_ref[...], preferred_element_type=f32))
    gate = _rb(gpre * jax.nn.sigmoid(gpre))
    up = _rb(jnp.dot(xsel, wu_ref[...], preferred_element_type=f32))
    y = _rb(jnp.dot((gate * up).astype(bf16), wd_ref[...], preferred_element_type=f32))
    rsel = _rb(jax.nn.sigmoid(jnp.where(row16 == 0, m1, m2)))
    y = _rb(y * rsel)
    y1 = y[0:1, :]
    y2 = y[1:2, :]
    for idx in (i1, i2):
        base = pl.multiple_of((idx // 16) * 16, 16)
        hg = h_ref[pl.ds(base, 16), :]
        hng = _rb(_layernorm(hg))
        t = row16 + base
        upd = jnp.where(t == i1, y1, jnp.where(t == i2, y2, 0.0))
        o_ref[pl.ds(base, 16), :] = (hg + _rb(hng + upd)).astype(bf16)


@jax.jit
def pallas_sequential_preLN__mha_block__moe_arch_mod__prompt_kernel(
    A_x, A_wqkv, A_wo, B_x, B_w_r, B_w_gate, B_w_up, B_w_down,
):
    B, S, D = A_x.shape
    F = B_w_gate.shape[1]
    assert B == 1 and D == H * DH and S % TQ == 0 and S % TB == 0
    vmem = pl.BlockSpec(memory_space=pltpu.VMEM)
    hbm = pl.BlockSpec(memory_space=pl.ANY)
    NV = S // CK * 16
    out = pl.pallas_call(
        _kernel,
        out_shape=jax.ShapeDtypeStruct((S, D), A_x.dtype),
        in_specs=[vmem, vmem, vmem, hbm, hbm, hbm, hbm],
        out_specs=vmem,
        scratch_shapes=[
            pltpu.VMEM((H // HG, S // 2, 128), u32),
            pltpu.VMEM((H // HG, NV // 2, 128), u32),
            pltpu.VMEM((D, NV, 128), f32),
            pltpu.VMEM((D // 2, S), u32),
            pltpu.VMEM((D // 2, S), u32),
            pltpu.VMEM((D // 2, S), u32),
            pltpu.VMEM((H, S), f32),
            pltpu.VMEM((S, D), f32),
            pltpu.VMEM((8, TB), f32),
            pltpu.VMEM((2 * D, D), bf16),
            pltpu.VMEM((D, D), bf16),
            pltpu.VMEM((D, F), bf16),
            pltpu.VMEM((D, F), bf16),
            pltpu.VMEM((F, D), bf16),
            pltpu.SemaphoreType.DMA((4,)),
        ] + [pltpu.VMEM((CK // 2, TQ), u32)] * RING + [pltpu.VMEM((DH, 8, TQ), f32)] * HG,
        compiler_params=pltpu.CompilerParams(vmem_limit_bytes=120 * 1024 * 1024),
    )(A_x.reshape(S, D), A_wqkv, jnp.broadcast_to(B_w_r.reshape(1, D), (16, D)), A_wo, B_w_gate, B_w_up, B_w_down)
    return out.reshape(B, S, D)
```

```python
import math

import jax
import jax.numpy as jnp
from jax import lax
import jax.experimental.pallas as pl
import jax.experimental.pallas.tpu as pltpu

f32, bf16, u32, i32 = jnp.float32, jnp.bfloat16, jnp.uint32, jnp.int32

H = 32
DH = 16
HG = 8
TQ = 512
CK = 128
VK = 16
MK = CK - VK
LAG = 4
RING = 8
TP = 2 * CK
EPS = 1e-5
L_LO, L_HI = 2.0 ** -60, 2.0 ** 60
QS0 = 4


def _rb(x):
    return x.astype(bf16).astype(f32)


def _ln_mean(x):
    return jnp.sum(x, axis=-1, keepdims=True) * (1.0 / x.shape[-1])


def _ln_finish(x, mean):
    xc = x - mean
    var = jnp.sum(xc * xc, axis=-1, keepdims=True) * (1.0 / x.shape[-1])
    return xc * lax.rsqrt(var + EPS)


def _layernorm(x):
    return _ln_finish(x, _ln_mean(x))


def _layernorm_bf16(x):
    mean = _ln_mean(x)
    xc = x - mean
    var = jnp.sum(xc * xc, axis=-1, keepdims=True) * (1.0 / x.shape[-1])
    v = _rb(_rb(var) + EPS)
    den = _rb(v * lax.rsqrt(v))
    inv = pl.reciprocal(den, approx=True)
    inv = inv * (2.0 - den * inv)
    return _rb(x - _rb(mean)) * inv


def _pack(x):
    return pltpu.bitcast(x.astype(bf16), u32)


def _unpack(x):
    return pltpu.bitcast(x, bf16)


def _kernel(x_hbm, wqkv_hbm, wr_ref, wo_hbm, wg_hbm, wu_hbm, wd_hbm, o_hbm,
            x_ref, xn_ref, wqkv_ref, wt_ref, kp_ref, kv_ref, kb_ref, qp_ref, vp_ref, op_ref,
            l_ref, h_ref, r_ref, o_ref, wo_ref, wg_ref, wu_ref, wd_ref,
            xsem, wsem, osem, *stage):
    pt_refs = stage[:RING]
    qs_refs = stage[RING:]
    S, D = x_ref.shape
    NQ = S // TQ
    NC = S // CK
    NG = H // HG
    NP = S // TP
    NV = NC * VK
    MR = 2 * MK

    HB = NP // 2

    def x_copy(n):
        rows = pl.ds(0, NV) if n == 0 else pl.ds(NV + (n - 1) * HB * MR, HB * MR)
        return pltpu.make_async_copy(x_hbm.at[rows, :], x_ref.at[rows, :], xsem.at[n])

    def w_copy(n):
        if n < 3:
            cols = pl.ds(n * D, D)
            return pltpu.make_async_copy(wqkv_hbm.at[:, cols], wqkv_ref.at[:, cols], wsem.at[n])
        src, dst = ((wo_hbm, wo_ref), (wg_hbm, wg_ref), (wu_hbm, wu_ref), (wd_hbm, wd_ref))[n - 3]
        return pltpu.make_async_copy(src, dst, wsem.at[n])

    x_copy(0).start()
    w_copy(1).start()
    x_copy(1).start()
    x_copy(2).start()
    w_copy(0).start()
    w_copy(2).start()

    def bcast_keys(jds):
        for jd in jds:
            for c in range(NC):
                for g in range(NG):
                    src = kv_ref[g, c * 8:(c + 1) * 8, :]
                    if isinstance(jd, int):
                        col = jnp.broadcast_to(src[:, jd:jd + 1], (8, 128))
                    else:
                        col = jnp.take_along_axis(src, jnp.full((8, 128), jd, i32), axis=1)
                    kb_ref[g * 128 + jd, c * VK:(c + 1) * VK, :] = _unpack(col).astype(f32)

    def k_proj(b):
        al = (lambda v, m: v) if isinstance(b, int) else pl.multiple_of
        xu = jnp.concatenate(
            [xn_ref[pl.ds(al((2 * b + cc) * (CK // 2) + VK // 2, 8), MK // 2), :]
             for cc in range(2)], axis=0)
        k = jnp.dot(_unpack(xu), wqkv_ref[:, D:2 * D], preferred_element_type=f32)
        for g in range(NG):
            kp_ref[g, pl.ds(al(b * MK, 8), MK), :] = _pack(k[:, g * 128:(g + 1) * 128])

    def ln_blocks(blocks, jds, extra=None):
        xs = [x_ref[NV + b * MR:NV + (b + 1) * MR, :].astype(f32) for b in blocks]

        def finish(ns, means):
            for n, m in zip(ns, means):
                xu = pltpu.bitcast(_ln_finish(xs[n], m).astype(bf16), u32)
                for cc in range(2):
                    r0 = (2 * blocks[n] + cc) * (CK // 2) + VK // 2
                    xn_ref[r0:r0 + MK // 2, :] = xu[cc * (MK // 2):(cc + 1) * (MK // 2)]

        q1, q2 = 1, 4
        m01 = [_ln_mean(xs[0]), _ln_mean(xs[1])]
        bcast_keys(jds[:q1])
        finish((0, 1), m01)
        m23 = [_ln_mean(xs[2]), _ln_mean(xs[3])]
        bcast_keys(jds[q1:q2])
        finish((2, 3), m23)
        if extra is not None:
            extra()
        bcast_keys(jds[q2:])

    DPRE = 4
    KL = 0
    pre_jds = [j * DH + d for d in range(DPRE) for j in range(HG)]
    n2, n3 = 3, 13

    x_copy(0).wait()
    xn0 = _layernorm(x_ref[0:NV, :].astype(f32)).astype(bf16)
    xu0 = pltpu.bitcast(xn0, u32)
    for c in range(NC):
        xn_ref[c * (CK // 2):c * (CK // 2) + VK // 2, :] = xu0[c * 8:(c + 1) * 8]
    w_copy(1).wait()
    kv = jnp.dot(xn0, wqkv_ref[:, D:2 * D], preferred_element_type=f32)
    for g in range(NG):
        kv_ref[g] = _pack(kv[:, g * 128:(g + 1) * 128])
    bcast_keys(pre_jds[:n2])
    x_copy(1).wait()
    ln_blocks(list(range(HB)), pre_jds[n2:n2 + n3])
    K3 = 3
    for b in range(K3):
        k_proj(b)
    x_copy(2).wait()
    w_copy(0).wait()
    w_copy(2).wait()
    for n in range(3, 7):
        w_copy(n).start()

    def transpose_weights():
        wt_ref[0:D, :] = wqkv_ref[:, 0:D].astype(f32).T.astype(bf16)
        wt_ref[D:2 * D, :] = wqkv_ref[:, 2 * D:3 * D].astype(f32).T.astype(bf16)

    ln_blocks(list(range(HB, NP)), pre_jds[n2 + n3:], transpose_weights)
    for b in range(K3, NP - KL):
        k_proj(b)
    qscale = (DH ** -0.5) * math.log2(math.e)

    PB = 2

    def proj(t, carry):
        for r in range(PB):
            b = t * PB + r
            bcast_keys([b * DH + d for d in range(DPRE, DH)])
            xp = _unpack(xn_ref[pl.ds(pl.multiple_of(b * (TP // 2), TP // 2), TP // 2), :])
            qv = lax.dot_general(wt_ref[...], xp, (((1,), (1,)), ((), ())),
                                 preferred_element_type=f32)
            cols = pl.ds(pl.multiple_of(b * TP, TP), TP)
            qp_ref[:, cols] = _pack(_rb(qv[0:D]) * qscale)
            vp_ref[:, cols] = _pack(qv[D:2 * D])
        return carry

    lax.fori_loop(0, NP // PB, proj, 0)

    NI = NQ * NG

    def unit_index(i, j):
        qb = i // NG
        h = (i % NG) * HG + j
        return h, pl.multiple_of(h * 8, 8), pl.ds(pl.multiple_of(qb * TQ, TQ), TQ)

    def stage_q(i, j, lo, hi):
        _, h8, cols = unit_index(i, j)
        qf = _unpack(qp_ref[pl.ds(h8, 8), cols]).astype(f32)
        for d in range(lo, hi):
            qs_refs[j][d] = jnp.broadcast_to(qf[d:d + 1, :], (8, TQ))

    def pv_step(i, j, c, slot, zz, acc, l8, link=None):
        h, h8, cols = unit_index(i, j)
        vt = _unpack(vp_ref[pl.ds(h8, 8), c * CK:(c + 1) * CK])
        d = jnp.dot(vt, _unpack(pt_refs[slot][pl.ds(zz, CK // 2), :]),
                    preferred_element_type=f32)
        if acc is None:
            acc = d if link is None else jnp.where(link[0], link[1], d)
        else:
            acc = acc + d
        if c == NC - 1:
            if not 1:
                l8 = inv_denominator(i, j, l8)
            op_ref[pl.ds(h8, 8), cols] = _pack(acc * jnp.concatenate([l8, l8], axis=0))
        return acc

    def inv_denominator(i, j, l8):
        h, _, cols = unit_index(i, j)
        l = jnp.sum(l8, axis=0, keepdims=True)
        l_ref[pl.ds(h, 1), cols] = l
        inv = pl.reciprocal(l, approx=True)
        inv = inv * (2.0 - l * inv)
        return jnp.broadcast_to(inv, l8.shape)

    def fast_group(i, carry):
        g = i % NG
        ip = (i + NI - 1) % NI
        inx = jnp.minimum(i + 1, NI - 1)
        z1 = lax.shift_right_logical(i, 20)
        zz = pl.multiple_of(z1 * 8, 8)
        zt = [lax.shift_right_logical(i, 21 + (t // 4)) for t in range(TQ // 128)]
        never = lax.broadcasted_iota(i32, (VK, 128), 0) < z1
        never_wide = lax.broadcasted_iota(i32, (DH, TQ), 0) < z1
        acc = {-1: carry[0]}
        l8 = {-1: carry[1]}
        pend = [(-1, c, (c + NC * (HG - 1)) % RING) for c in range(NC - LAG, NC)]

        prev = None
        for j in range(HG):
            h, h8, cols = unit_index(i, j)
            qrow = qp_ref[pl.ds(h8, 8), cols]
            z = jnp.zeros_like(qrow)
            w = _unpack(jnp.concatenate([qrow if b == j else z for b in range(HG)], axis=0))
            acc[j] = None
            l8[j] = None
            jn = (j + 1) % HG
            for c in range(NC):
                slot = (j * NC + c) % RING
                base = c * (MK // 2)
                kc = _unpack(jnp.concatenate(
                    [kp_ref[g, base + b * 8:base + (b + 1) * 8, :] for b in range(6, -1, -1)],
                    axis=0))
                s = jnp.dot(kc, w, preferred_element_type=f32)
                p = jnp.exp2(s)
                cl = jnp.sum(p.reshape(MK // 8, 8, TQ), axis=0)
                l8[j] = cl if l8[j] is None else l8[j] + cl
                for b in range(7):
                    pt_refs[slot][(7 - b) * 8:(8 - b) * 8, :] = _pack(p[b * 16:(b + 1) * 16, :])
                pend.append((j, c, slot))
                pj, pc, pslot = pend.pop(0)
                link = (never_wide, acc[pj - 1]) if (pc == 0 and 1) else None
                acc[pj] = pv_step(ip if pj < 0 else i, pj % HG, pc, pslot, zz, acc[pj], l8[pj],
                                  link)

                tie = None
                if c - QS0 in (1, 3, 5, 7):
                    tie = qs_refs[jn][z1, :, 0:128]
                    tie = jnp.concatenate([tie, tie], axis=0)
                if not 1:
                    prev = None
                tiles = []
                KO = 2
                for t in range(TQ // 128):
                    a = None
                    for d in range(DH):
                        kb = kb_ref[h * DH + d + zt[t], c * VK:(c + 1) * VK, :]
                        qd = qs_refs[j][z1 + d, :, t * 128:(t + 1) * 128]
                        pr = kb * jnp.concatenate([qd, qd], axis=0)
                        if d == 0 and t == 0 and tie is not None:
                            pr = jnp.where(never, tie, pr)
                        a = pr if a is None else a + pr
                        if d == KO and prev is not None:
                            a = jnp.where(never, prev, a)
                    tiles.append(a)
                    prev = a
                p = jnp.exp2(jnp.concatenate(tiles, axis=1))
                l8[j] = l8[j] + (p[0:8] + p[8:16])
                pt_refs[slot][0:8, :] = _pack(p)
                if c == NC - 1 and 1:
                    l8[j] = inv_denominator(i, j, l8[j])
                if c - QS0 in (0, 2, 4, 6):
                    q4 = (c - QS0) * 2
                    stage_q(i if jn else inx, jn, q4, q4 + 4)
        return acc[HG - 1], l8[HG - 1]

    stage_q(0, 0, 0, DH)
    for c in range(NC - LAG, NC):
        pt_refs[(c + NC * (HG - 1)) % RING][...] = jnp.zeros((CK // 2, TQ), u32)
    acc, l8 = lax.fori_loop(0, NI, fast_group,
                            (jnp.zeros((DH, TQ), f32), jnp.ones((8, TQ), f32)))
    for c in range(NC - LAG, NC):
        acc = pv_step(NI - 1, HG - 1, c, (c + NC * (HG - 1)) % RING, 0, acc, l8)

    l_all = l_ref[...]
    safe = jnp.logical_and(jnp.min(l_all) >= L_LO, jnp.max(l_all) <= L_HI)
    @pl.when(jnp.logical_not(safe))
    def _():
        def unit(u, carry):
            qb = u // H
            h = u % H
            g = h // HG
            j = h % HG
            cols = pl.ds(pl.multiple_of(qb * TQ, TQ), TQ)
            h8 = pl.multiple_of(h * 8, 8)
            qrow = qp_ref[pl.ds(h8, 8), cols]
            z = jnp.zeros_like(qrow)
            w = _unpack(jnp.concatenate(
                [jnp.where(j == b, qrow, z) for b in range(HG)], axis=0))

            def scores(c):
                kc = jnp.concatenate(
                    [kv_ref[g, pl.ds(pl.multiple_of(c * 8, 8), 8), :],
                     kp_ref[g, pl.ds(pl.multiple_of(c * (MK // 2), 8), MK // 2), :]], axis=0)
                return jnp.dot(_unpack(kc), w, preferred_element_type=f32)

            def max_body(c, m):
                return jnp.maximum(m, jnp.max(scores(c), axis=0, keepdims=True))

            m = lax.fori_loop(0, NC, max_body, jnp.full((1, TQ), -jnp.inf, f32))

            def sum_body(c, la):
                l, a = la
                p = jnp.exp2(scores(c) - m)
                vt = _unpack(vp_ref[pl.ds(h8, 8), pl.ds(pl.multiple_of(c * CK, CK), CK)])
                a = a + jnp.dot(vt, p.astype(bf16), preferred_element_type=f32)
                return l + jnp.sum(p, axis=0, keepdims=True), a

            l, a = lax.fori_loop(0, NC, sum_body,
                                 (jnp.zeros((1, TQ), f32), jnp.zeros((DH, TQ), f32)))
            op_ref[pl.ds(h8, 8), cols] = _pack(a * (1.0 / l))
            return carry

        lax.fori_loop(0, NQ * H, unit, 0)

    def out_copy(n):
        rows = pl.ds(0, NV) if n == NP else pl.ds(NV + n * MR, MR)
        return pltpu.make_async_copy(o_ref.at[rows, :], o_hbm.at[rows, :], osem.at[n])

    def token_spans(b):
        spans = []
        for cc in range(2):
            c = 2 * b + cc
            spans += [(cc * CK, c * VK, VK), (cc * CK + VK, NV + c * MK, MK)]
        return spans

    w_copy(3).wait()
    wr = wr_ref[...]

    def out_proj(b):
        ot = _unpack(op_ref[:, b * TP:(b + 1) * TP])
        return lax.dot_general(ot, wo_ref[...], (((0,), (0,)), ((), ())),
                               preferred_element_type=f32)

    def residual_ln(b, attn):
        xb = jnp.concatenate([x_ref[t0:t0 + n, :].astype(f32) for _, t0, n in token_spans(b)], axis=0)
        h = _rb(xb + _rb(attn))
        hn = _layernorm_bf16(h).astype(bf16)
        o = h + hn.astype(f32)
        for p0, t0, n in token_spans(b):
            h_ref[t0:t0 + n, :] = h[p0:p0 + n]
            o_ref[t0:t0 + n, :] = o[p0:p0 + n].astype(bf16)
        out_copy(b).start()
        return hn

    def router(b, hn):
        r = lax.dot_general(wr, hn, (((1,), (1,)), ((), ())), preferred_element_type=f32)
        r_ref[b:b + 1, :] = _rb(r[0:1, :]) + 0.0

    attn = out_proj(0)
    hn_prev = None
    for b in range(NP):
        attn_next = out_proj(b + 1) if b + 1 < NP else None
        if hn_prev is not None:
            router(b - 1, hn_prev)
        hn_prev = residual_ln(b, attn)
        attn = attn_next
    router(NP - 1, hn_prev)
    out_copy(NP).start()

    r = r_ref[0:NP, :]
    pos = lax.broadcasted_iota(i32, r.shape, 0) * TP + lax.broadcasted_iota(i32, r.shape, 1)
    ch = pos // CK
    off = pos % CK
    tok = jnp.where(off < VK, ch * VK + off, NV + ch * MK + off - VK)
    bits = pltpu.bitcast(r, i32)
    mono = jnp.where(bits < 0, bits ^ 0x7FFF0000, bits)
    key = mono | (S - 1 - tok)
    k1 = jnp.max(key)
    k2 = jnp.max(jnp.where(key == k1, jnp.iinfo(jnp.int32).min, key))
    i1 = S - 1 - (k1 & 0xFFFF)
    i2 = S - 1 - (k2 & 0xFFFF)

    row16 = lax.broadcasted_iota(i32, (16, D), 0)
    ksel = jnp.where(row16 == 0, k1, k2) & jnp.int32(-65536)
    rtop = pltpu.bitcast(jnp.where(ksel < 0, ksel ^ 0x7FFF0000, ksel), f32)
    h1 = h_ref[pl.ds(i1, 1), :]
    h2 = h_ref[pl.ds(i2, 1), :]
    hsel = jnp.where(row16 == 0, h1, h2)
    xsel = _layernorm_bf16(hsel).astype(bf16)
    w_copy(4).wait()
    w_copy(5).wait()
    w_copy(6).wait()
    gpre = _rb(jnp.dot(xsel, wg_ref[...], preferred_element_type=f32))
    gate = _rb(gpre * jax.nn.sigmoid(gpre))
    up = _rb(jnp.dot(xsel, wu_ref[...], preferred_element_type=f32))
    y = _rb(jnp.dot((gate * up).astype(bf16), wd_ref[...], preferred_element_type=f32))
    y = _rb(y * _rb(jax.nn.sigmoid(rtop)))
    y1 = y[0:1, :]
    y2 = y[1:2, :]
    for n in range(NP + 1):
        out_copy(n).wait()
    bases = [pl.multiple_of((idx // 16) * 16, 16) for idx in (i1, i2)]
    for base in bases:
        hg = h_ref[pl.ds(base, 16), :]
        hng = _rb(_layernorm_bf16(hg))
        t = row16 + base
        upd = jnp.where(t == i1, y1, jnp.where(t == i2, y2, 0.0))
        o_ref[pl.ds(base, 16), :] = (hg + _rb(hng + upd)).astype(bf16)
    patch = [pltpu.make_async_copy(o_ref.at[pl.ds(base, 16), :], o_hbm.at[pl.ds(base, 16), :],
                                   osem.at[n]) for n, base in enumerate(bases)]
    patch[0].start()

    @pl.when(bases[0] != bases[1])
    def _():
        patch[1].start()
        patch[1].wait()

    patch[0].wait()


@jax.jit
def pallas_sequential_preLN__mha_block__moe_arch_mod__prompt_kernel(
    A_x, A_wqkv, A_wo, B_x, B_w_r, B_w_gate, B_w_up, B_w_down,
):
    B, S, D = A_x.shape
    F = B_w_gate.shape[1]
    assert B == 1 and D == H * DH and S % TQ == 0 and S // TP == 8
    vmem = pl.BlockSpec(memory_space=pltpu.VMEM)
    hbm = pl.BlockSpec(memory_space=pl.ANY)
    NC = S // CK
    NV = NC * VK
    out = pl.pallas_call(
        _kernel,
        out_shape=jax.ShapeDtypeStruct((S, D), A_x.dtype),
        in_specs=[hbm, hbm, vmem, hbm, hbm, hbm, hbm],
        out_specs=hbm,
        scratch_shapes=[
            pltpu.VMEM((S, D), bf16),
            pltpu.VMEM((S // 2, D), u32),
            pltpu.VMEM((D, 3 * D), bf16),
            pltpu.VMEM((2 * D, D), bf16),
            pltpu.VMEM((H // HG, NC * MK // 2, 128), u32),
            pltpu.VMEM((H // HG, NV // 2, 128), u32),
            pltpu.VMEM((D, NV, 128), f32),
            pltpu.VMEM((D // 2, S), u32),
            pltpu.VMEM((D // 2, S), u32),
            pltpu.VMEM((D // 2, S), u32),
            pltpu.VMEM((H, S), f32),
            pltpu.VMEM((S, D), f32),
            pltpu.VMEM((16, TP), f32),
            pltpu.VMEM((S, D), bf16),
            pltpu.VMEM((D, D), bf16),
            pltpu.VMEM((D, F), bf16),
            pltpu.VMEM((D, F), bf16),
            pltpu.VMEM((F, D), bf16),
            pltpu.SemaphoreType.DMA((3,)),
            pltpu.SemaphoreType.DMA((7,)),
            pltpu.SemaphoreType.DMA((S // TP + 1,)),
        ] + [pltpu.VMEM((CK // 2, TQ), u32)] * RING + [pltpu.VMEM((DH, 8, TQ), f32)] * HG,
        compiler_params=pltpu.CompilerParams(vmem_limit_bytes=120 * 1024 * 1024),
    )(A_x.reshape(S, D), A_wqkv, jnp.broadcast_to(B_w_r.reshape(1, D), (16, D)),
      A_wo, B_w_gate, B_w_up, B_w_down)
    return out.reshape(B, S, D)
```

```python
import math

import jax
import jax.numpy as jnp
from jax import lax
import jax.experimental.pallas as pl
import jax.experimental.pallas.tpu as pltpu

f32, bf16, u32, i32 = jnp.float32, jnp.bfloat16, jnp.uint32, jnp.int32

H = 32
DH = 16
HG = 8
TQ = 512
CK = 128
VK = 16
MK = CK - VK
LAG = 4
RING = 8
TP = 2 * CK
EPS = 1e-5
BF16_MAX = 3.3895313892515355e38
F32_TINY = 2.0 ** -126
L_LO, L_HI = 2.0 ** -60, 2.0 ** 60


def _rb(x):
    return x.astype(bf16).astype(f32)


def _mean(x):
    return jnp.sum(x, axis=-1, keepdims=True) * (1.0 / x.shape[-1])


def _layernorm(x):
    xc = x - _mean(x)
    return xc * lax.rsqrt(_mean(xc * xc) + EPS)


def _layernorm_bf16(x):
    mean = _mean(x)
    xc = x - mean
    v = _rb(_rb(_mean(xc * xc)) + EPS)
    den = _rb(v * lax.rsqrt(v))
    inv = pl.reciprocal(den, approx=True)
    inv = inv * (2.0 - den * inv)
    return (x - _rb(mean)) * inv


def _pack(x):
    return pltpu.bitcast(x.astype(bf16), u32)


def _unpack(x):
    return pltpu.bitcast(x, bf16)


def _kernel(x_hbm, wqkv_hbm, wr_hbm, wo_hbm, wg_hbm, wu_hbm, wd_hbm, o_hbm,
            x_ref, xn_ref, wqkv_ref, wt_ref, kp_ref, kv_ref, kb_ref, qp_ref, vp_ref, op_ref,
            l_ref, h_ref, hn_ref, o_ref, wo_ref, wg_ref, wu_ref, wd_ref, wr_ref,
            xsem, wsem, osem, *stage):
    pt_refs = stage[:RING]
    qs_refs = stage[RING:]
    S, D = x_ref.shape
    NQ = S // TQ
    NC = S // CK
    NG = H // HG
    NP = S // TP
    HP = NP // 2
    NV = NC * VK
    MR = 2 * MK

    def x_copy(n):
        rows = pl.ds(0, NV) if n == 0 else pl.ds(NV + (n - 1) * HP * MR, HP * MR)
        return pltpu.make_async_copy(x_hbm.at[rows, :], x_ref.at[rows, :], xsem.at[n])

    def w_copy(n):
        if n < 3:
            cols = pl.ds(n * D, D)
            return pltpu.make_async_copy(wqkv_hbm.at[:, cols], wqkv_ref.at[:, cols], wsem.at[n])
        src, dst = ((wo_hbm, wo_ref), (wg_hbm, wg_ref), (wu_hbm, wu_ref), (wd_hbm, wd_ref),
                    (wr_hbm, wr_ref.at[pl.ds(0, D)]))[n - 3]
        return pltpu.make_async_copy(src, dst, wsem.at[n])

    x_copy(0).start()
    w_copy(1).start()
    x_copy(1).start()
    x_copy(2).start()
    w_copy(0).start()
    w_copy(2).start()

    def bcast_keys(jds):
        for jd in jds:
            for c in range(NC):
                for g in range(NG):
                    col = jnp.broadcast_to(kv_ref[g, c * 8:(c + 1) * 8, jd:jd + 1], (8, 128))
                    kb_ref[g * 128 + jd, c * VK:(c + 1) * VK, :] = _unpack(col).astype(f32)

    def ln_block(b):
        xn = _layernorm(x_ref[NV + b * MR:NV + (b + 1) * MR, :].astype(f32))
        xu = _pack(xn)
        for cc in range(2):
            r0 = (2 * b + cc) * (CK // 2) + VK // 2
            xn_ref[r0:r0 + MK // 2, :] = xu[cc * (MK // 2):(cc + 1) * (MK // 2)]

    def k_proj(b):
        xu = jnp.concatenate(
            [xn_ref[(2 * b + cc) * (CK // 2) + VK // 2:(2 * b + cc + 1) * (CK // 2), :]
             for cc in range(2)], axis=0)
        k = jnp.dot(_unpack(xu), wqkv_ref[:, D:2 * D], preferred_element_type=f32)
        for g in range(NG):
            kp_ref[g, b * MK:(b + 1) * MK, :] = _pack(k[:, g * 128:(g + 1) * 128])

    early = 4
    jds = [j * DH + d for d in range(early) for j in range(HG)]

    x_copy(0).wait()
    xu0 = _pack(_layernorm(x_ref[0:NV, :].astype(f32)))
    for c in range(NC):
        xn_ref[c * (CK // 2):c * (CK // 2) + VK // 2, :] = xu0[c * 8:(c + 1) * 8]
    w_copy(1).wait()
    kv = jnp.dot(_unpack(xu0), wqkv_ref[:, D:2 * D], preferred_element_type=f32)
    for g in range(NG):
        kv_ref[g] = _pack(kv[:, g * 128:(g + 1) * 128])
    bcast_keys(jds[:3])
    x_copy(1).wait()
    for b in range(HP):
        ln_block(b)
    bcast_keys(jds[3:16])
    for b in range(HP - 1):
        k_proj(b)
    x_copy(2).wait()
    w_copy(0).wait()
    w_copy(2).wait()
    for n in range(3, 8):
        w_copy(n).start()
    for b in range(HP, NP):
        ln_block(b)
    wt_ref[0:D, :] = wqkv_ref[:, 0:D].astype(f32).T.astype(bf16)
    wt_ref[D:2 * D, :] = wqkv_ref[:, 2 * D:3 * D].astype(f32).T.astype(bf16)
    bcast_keys(jds[16:])
    for b in range(HP - 1, NP):
        k_proj(b)
    qscale = (DH ** -0.5) * math.log2(math.e)
    for b in range(NP):
        bcast_keys([b * DH + d for d in range(early, DH)])
        xp = _unpack(xn_ref[b * (TP // 2):(b + 1) * (TP // 2), :])
        qv = lax.dot_general(wt_ref[...], xp, (((1,), (1,)), ((), ())),
                             preferred_element_type=f32)
        qp_ref[:, b * TP:(b + 1) * TP] = _pack(qv[0:D] * qscale)
        vp_ref[:, b * TP:(b + 1) * TP] = _pack(qv[D:2 * D])

    NI = NQ * NG

    def unit_index(i, j):
        h = (i % NG) * HG + j
        return h, pl.multiple_of(h * 8, 8), pl.ds(pl.multiple_of((i // NG) * TQ, TQ), TQ)

    def stage_q(i, j, lo, hi):
        _, h8, cols = unit_index(i, j)
        qf = _unpack(qp_ref[pl.ds(h8, 8), cols]).astype(f32)
        for d in range(lo, hi):
            qs_refs[j][d] = jnp.broadcast_to(qf[d:d + 1, :], (8, TQ))

    def pv_step(i, j, c, row0, acc, inv_l, link=None):
        _, h8, cols = unit_index(i, j)
        vt = _unpack(vp_ref[pl.ds(h8, 8), c * CK:(c + 1) * CK])
        d = jnp.dot(vt, _unpack(pt_refs[c % RING][pl.ds(row0, CK // 2), :]),
                    preferred_element_type=f32)
        if acc is None:
            acc = jnp.where(link[0], link[1], d)
        else:
            acc = acc + d
        if c == NC - 1:
            op_ref[pl.ds(h8, 8), cols] = _pack(acc * jnp.concatenate([inv_l, inv_l], axis=0))
        return acc

    def inv_denominator(i, j, l8):
        h, _, cols = unit_index(i, j)
        l = jnp.sum(l8, axis=0, keepdims=True)
        l_ref[pl.ds(h, 1), cols] = l
        inv = pl.reciprocal(l, approx=True)
        inv = inv * (2.0 - l * inv)
        return jnp.broadcast_to(inv, l8.shape)

    def fast_group(i, carry):
        z1 = lax.shift_right_logical(i, 20)
        row0 = pl.multiple_of(z1 * 8, 8)
        never = lax.broadcasted_iota(i32, (VK, 128), 0) < z1
        never_wide = lax.broadcasted_iota(i32, (DH, TQ), 0) < z1
        g = i % NG
        grp = {j: i for j in range(HG)}
        grp[-1] = (i + NI - 1) % NI
        grp[HG] = jnp.minimum(i + 1, NI - 1)
        acc = {-1: carry[0]}
        l8 = {-1: carry[1]}
        pend = [(-1, c) for c in range(NC - LAG, NC)]
        prev = None
        for j in range(HG):
            h, h8, cols = unit_index(i, j)
            qrow = qp_ref[pl.ds(h8, 8), cols]
            z = jnp.zeros_like(qrow)
            w = _unpack(jnp.concatenate([qrow if b == j else z for b in range(HG)], axis=0))
            acc[j] = None
            l8[j] = None
            jn = (j + 1) % HG
            for c in range(NC):
                pt_ref = pt_refs[c % RING]
                base = c * (MK // 2)
                kc = _unpack(jnp.concatenate(
                    [kp_ref[g, base + b * 8:base + (b + 1) * 8, :] for b in range(6, -1, -1)],
                    axis=0))
                p = jnp.exp2(jnp.dot(kc, w, preferred_element_type=f32))
                cl = jnp.sum(p.reshape(MK // 8, 8, TQ), axis=0)
                l8[j] = cl if l8[j] is None else l8[j] + cl
                for b in range(7):
                    pt_ref[(7 - b) * 8:(8 - b) * 8, :] = _pack(p[b * 16:(b + 1) * 16, :])
                pend.append((j, c))
                pj, pc = pend.pop(0)
                link = (never_wide, acc[pj - 1]) if pc == 0 else None
                acc[pj] = pv_step(grp[pj], pj % HG, pc, row0, acc[pj], l8[pj], link)

                tie = None
                if c in (5, 7, 9, 11):
                    tie = qs_refs[jn][z1, :, 0:128]
                    tie = jnp.concatenate([tie, tie], axis=0)
                tiles = []
                for t in range(TQ // 128):
                    a = None
                    for d in range(DH):
                        kb = kb_ref[h * DH + d + z1, c * VK:(c + 1) * VK, :]
                        qd = qs_refs[j][z1 + d, :, t * 128:(t + 1) * 128]
                        pr = kb * jnp.concatenate([qd, qd], axis=0)
                        if d == 0 and t == 0 and tie is not None:
                            pr = jnp.where(never, tie, pr)
                        a = pr if a is None else a + pr
                        if d == 2 and prev is not None:
                            a = jnp.where(never, prev, a)
                    tiles.append(a)
                    prev = a
                p = jnp.exp2(jnp.concatenate(tiles, axis=1))
                l8[j] = l8[j] + (p[0:8] + p[8:16])
                pt_ref[0:8, :] = _pack(p)
                if c == NC - 1:
                    l8[j] = inv_denominator(i, j, l8[j])
                if c in (4, 6, 8, 10):
                    stage_q(grp[j + 1], jn, (c - 4) * 2, (c - 4) * 2 + 4)
        return acc[HG - 1], l8[HG - 1]

    stage_q(0, 0, 0, DH)
    for c in range(NC - LAG, NC):
        pt_refs[c % RING][...] = jnp.zeros((CK // 2, TQ), u32)
    acc, inv_l = lax.fori_loop(0, NI, fast_group,
                               (jnp.zeros((DH, TQ), f32), jnp.ones((8, TQ), f32)))
    for c in range(NC - LAG, NC):
        acc = pv_step(NI - 1, HG - 1, c, 0, acc, inv_l)

    l_all = l_ref[...]
    safe = jnp.logical_and(jnp.min(l_all) >= L_LO, jnp.max(l_all) <= L_HI)

    @pl.when(jnp.logical_not(safe))
    def _():
        def unit(u, carry):
            h = u % H
            g = h // HG
            j = h % HG
            cols = pl.ds(pl.multiple_of((u // H) * TQ, TQ), TQ)
            h8 = pl.multiple_of(h * 8, 8)
            qrow = qp_ref[pl.ds(h8, 8), cols]
            z = jnp.zeros_like(qrow)
            w = _unpack(jnp.concatenate(
                [jnp.where(j == b, qrow, z) for b in range(HG)], axis=0))

            def scores(c):
                kc = jnp.concatenate(
                    [kv_ref[g, pl.ds(pl.multiple_of(c * 8, 8), 8), :],
                     kp_ref[g, pl.ds(pl.multiple_of(c * (MK // 2), 8), MK // 2), :]], axis=0)
                return jnp.dot(_unpack(kc), w, preferred_element_type=f32)

            def max_body(c, m):
                return jnp.maximum(m, jnp.max(scores(c), axis=0, keepdims=True))

            m = lax.fori_loop(0, NC, max_body, jnp.full((1, TQ), -jnp.inf, f32))

            def sum_body(c, la):
                l, a = la
                p = jnp.exp2(scores(c) - m)
                vt = _unpack(vp_ref[pl.ds(h8, 8), pl.ds(pl.multiple_of(c * CK, CK), CK)])
                a = a + jnp.dot(vt, p.astype(bf16), preferred_element_type=f32)
                return l + jnp.sum(p, axis=0, keepdims=True), a

            l, a = lax.fori_loop(0, NC, sum_body,
                                 (jnp.zeros((1, TQ), f32), jnp.zeros((DH, TQ), f32)))
            op_ref[pl.ds(h8, 8), cols] = _pack(a * (1.0 / l))
            return carry

        lax.fori_loop(0, NQ * H, unit, 0)

    def out_copy(n):
        rows = pl.ds(0, NV) if n == NP else pl.ds(NV + n * MR, MR)
        return pltpu.make_async_copy(o_ref.at[rows, :], o_hbm.at[rows, :], osem.at[n])

    send_after = {7: range(0, 4), 13: range(4, 7), 15: range(7, NP + 1)}

    def token_spans(c):
        return ((0, c * VK, VK), (VK, NV + c * MK, MK))

    w_copy(3).wait()
    w_copy(7).wait()
    wr = jnp.broadcast_to(wr_ref[pl.ds(0, D)].astype(f32).reshape(1, D), (16, D)).astype(bf16)
    wo = wo_ref[...]

    def out_proj(c):
        ot = _unpack(op_ref[:, c * CK:(c + 1) * CK])
        return lax.dot_general(ot, wo, (((0,), (0,)), ((), ())),
                               preferred_element_type=f32)

    def residual_ln(c, attn):
        xb = jnp.concatenate(
            [x_ref[t0:t0 + n, :].astype(f32) for _, t0, n in token_spans(c)], axis=0)
        h = _rb(xb + attn)
        hn = _layernorm_bf16(h).astype(bf16)
        hnf = hn.astype(f32)
        o = h + hnf
        for p0, t0, n in token_spans(c):
            h_ref[t0:t0 + n, :] = h[p0:p0 + n]
            hn_ref[t0:t0 + n, :] = hnf[p0:p0 + n]
            o_ref[t0:t0 + n, :] = o[p0:p0 + n].astype(bf16)
        for n in send_after.get(c, ()):
            out_copy(n).start()
        return hn

    def router(c, hn):
        r = lax.dot_general(wr, hn, (((1,), (1,)), ((), ())), preferred_element_type=f32)
        r = jnp.clip(_rb(r[0:8, :]), -BF16_MAX, BF16_MAX)
        r = jnp.where(jnp.abs(r) < F32_TINY, F32_TINY, r)
        off = lax.broadcasted_iota(i32, r.shape, 1)
        tok = off + jnp.where(off < VK, c * VK, NV + c * MK - VK)
        key = pltpu.bitcast(r, i32) | jnp.where(r < 0, tok, S - 1 - tok)
        return pltpu.bitcast(key, f32)

    attn = out_proj(0)
    hn_prev = None
    keys = []
    for c in range(NC):
        attn_next = out_proj(c + 1) if c + 1 < NC else None
        if hn_prev is not None:
            keys.append(router(c - 1, hn_prev))
        hn_prev = residual_ln(c, attn)
        attn = attn_next
    keys.append(router(NC - 1, hn_prev))

    top, sec = keys[0], jnp.full(keys[0].shape, -jnp.inf, f32)
    for k in keys[1:]:
        sec = jnp.maximum(sec, jnp.minimum(top, k))
        top = jnp.maximum(top, k)
    k1 = jnp.max(top, axis=1, keepdims=True)
    k2 = jnp.max(jnp.where(top == k1, sec, top), axis=1, keepdims=True)

    def decode(k):
        bits = pltpu.bitcast(jnp.broadcast_to(k, (8, 128)), i32)
        low = bits & 0xFFFF
        tok = jnp.where(bits < 0, low, S - 1 - low)
        score = pltpu.bitcast(bits & jnp.int32(-65536), f32)
        return jnp.clip(tok[0, 0], 0, S - 1), score[0:1, 0:1]

    i1, r1 = decode(k1)
    i2, r2 = decode(k2)
    row16 = lax.broadcasted_iota(i32, (16, D), 0)
    first = row16 == 0
    hsel = jnp.where(first, h_ref[pl.ds(i1, 1), :], h_ref[pl.ds(i2, 1), :])
    xsel = jnp.where(first, hn_ref[pl.ds(i1, 1), :], hn_ref[pl.ds(i2, 1), :])
    xs = xsel.astype(bf16)
    w_copy(4).wait()
    w_copy(5).wait()
    w_copy(6).wait()
    gpre = _rb(jnp.dot(xs, wg_ref[...], preferred_element_type=f32))
    gate = _rb(gpre * jax.nn.sigmoid(gpre))
    up = _rb(jnp.dot(xs, wu_ref[...], preferred_element_type=f32))
    y = _rb(jnp.dot((gate * up).astype(bf16), wd_ref[...], preferred_element_type=f32))
    y = _rb(y * _rb(jax.nn.sigmoid(jnp.where(first, r1, r2))))
    osel = hsel + _rb(xsel + y)
    for n in range(NP + 1):
        out_copy(n).wait()
    bases = [pl.multiple_of(lax.shift_right_logical(idx, 4) * 16, 16) for idx in (i1, i2)]
    olds = [o_ref[pl.ds(base, 16), :].astype(f32) for base in bases]
    for base, old in zip(bases, olds):
        t = row16 + base
        new = jnp.where(t == i1, osel[0:1, :], jnp.where(t == i2, osel[1:2, :], old))
        o_ref[pl.ds(base, 16), :] = new.astype(bf16)
    patch = [pltpu.make_async_copy(o_ref.at[pl.ds(base, 16), :], o_hbm.at[pl.ds(base, 16), :],
                                   osem.at[n]) for n, base in enumerate(bases)]
    patch[0].start()

    @pl.when(bases[0] != bases[1])
    def _():
        patch[1].start()
        patch[1].wait()

    patch[0].wait()


@jax.jit
def pallas_sequential_preLN__mha_block__moe_arch_mod__prompt_kernel(
    A_x: jax.Array,
    A_wqkv: jax.Array,
    A_wo: jax.Array,
    B_x: jax.Array,
    B_w_r: jax.Array,
    B_w_gate: jax.Array,
    B_w_up: jax.Array,
    B_w_down: jax.Array,
):
    B, S, D = A_x.shape
    F = B_w_gate.shape[1]
    assert B == 1 and D == H * DH and S == 2048
    hbm = pl.BlockSpec(memory_space=pl.ANY)
    NC = S // CK
    NV = NC * VK
    out = pl.pallas_call(
        _kernel,
        out_shape=jax.ShapeDtypeStruct((S, D), A_x.dtype),
        in_specs=[hbm] * 7,
        out_specs=hbm,
        scratch_shapes=[
            pltpu.VMEM((S, D), bf16),
            pltpu.VMEM((S // 2, D), u32),
            pltpu.VMEM((D, 3 * D), bf16),
            pltpu.VMEM((2 * D, D), bf16),
            pltpu.VMEM((H // HG, NC * MK // 2, 128), u32),
            pltpu.VMEM((H // HG, NV // 2, 128), u32),
            pltpu.VMEM((D, NV, 128), f32),
            pltpu.VMEM((D // 2, S), u32),
            pltpu.VMEM((D // 2, S), u32),
            pltpu.VMEM((D // 2, S), u32),
            pltpu.VMEM((H, S), f32),
            pltpu.VMEM((S, D), f32),
            pltpu.VMEM((S, D), f32),
            pltpu.VMEM((S, D), bf16),
            pltpu.VMEM((D, D), bf16),
            pltpu.VMEM((D, F), bf16),
            pltpu.VMEM((D, F), bf16),
            pltpu.VMEM((F, D), bf16),
            pltpu.VMEM((16 * D,), bf16),
            pltpu.SemaphoreType.DMA((3,)),
            pltpu.SemaphoreType.DMA((8,)),
            pltpu.SemaphoreType.DMA((S // TP + 1,)),
        ] + [pltpu.VMEM((CK // 2, TQ), u32)] * RING + [pltpu.VMEM((DH, 8, TQ), f32)] * HG,
        compiler_params=pltpu.CompilerParams(vmem_limit_bytes=120 * 1024 * 1024),
    )(A_x.reshape(S, D), A_wqkv, B_w_r, A_wo, B_w_gate, B_w_up, B_w_down)
    return out.reshape(B, S, D)
```

```python
import math

import jax
import jax.numpy as jnp
from jax import lax
import jax.experimental.pallas as pl
import jax.experimental.pallas.tpu as pltpu

f32, bf16, u32, i32 = jnp.float32, jnp.bfloat16, jnp.uint32, jnp.int32

H = 32
DH = 16
HG = 8
TQ = 512
CK = 128
VK = 16
MK = CK - VK
LAG = 4
RING = 8
TP = 2 * CK
EPS = 1e-5
BF16_MAX = 3.3895313892515355e38
F32_TINY = 2.0 ** -126
L_LO, L_HI = 2.0 ** -60, 2.0 ** 60


def _rb(x):
    return x.astype(bf16).astype(f32)


def _mean(x):
    return jnp.sum(x, axis=-1, keepdims=True) * (1.0 / x.shape[-1])


def _layernorm(x):
    xc = x - _mean(x)
    return xc * lax.rsqrt(_mean(xc * xc) + EPS)


def _layernorm_bf16(x):
    mean = _mean(x)
    xc = x - mean
    v = _rb(_rb(_mean(xc * xc)) + EPS)
    den = _rb(v * lax.rsqrt(v))
    inv = pl.reciprocal(den, approx=True)
    inv = inv * (2.0 - den * inv)
    return (x - _rb(mean)) * inv


def _pack(x):
    return pltpu.bitcast(x.astype(bf16), u32)


def _unpack(x):
    return pltpu.bitcast(x, bf16)


def _kernel(x_hbm, wqkv_hbm, wr_hbm, wo_hbm, wg_hbm, wu_hbm, wd_hbm, o_hbm,
            x_ref, xn_ref, wqkv_ref, wt_ref, kp_ref, kv_ref, kb_ref, qp_ref, vp_ref, op_ref,
            l_ref, h_ref, hn_ref, o_ref, wo_ref, wg_ref, wu_ref, wd_ref, wr_ref,
            xsem, wsem, osem, *stage):
    pt_refs = stage[:RING]
    qs_refs = stage[RING:]
    S, D = x_ref.shape
    NQ = S // TQ
    NC = S // CK
    NG = H // HG
    NP = S // TP
    HP = NP // 2
    NV = NC * VK
    MR = 2 * MK

    def x_copy(n):
        rows = pl.ds(0, NV) if n == 0 else pl.ds(NV + (n - 1) * HP * MR, HP * MR)
        return pltpu.make_async_copy(x_hbm.at[rows, :], x_ref.at[rows, :], xsem.at[n])

    def w_copy(n):
        if n < 3:
            cols = pl.ds(n * D, D)
            return pltpu.make_async_copy(wqkv_hbm.at[:, cols], wqkv_ref.at[:, cols], wsem.at[n])
        src, dst = ((wo_hbm, wo_ref), (wg_hbm, wg_ref), (wu_hbm, wu_ref), (wd_hbm, wd_ref),
                    (wr_hbm, wr_ref.at[pl.ds(0, D)]))[n - 3]
        return pltpu.make_async_copy(src, dst, wsem.at[n])

    x_copy(0).start()
    w_copy(1).start()
    x_copy(1).start()
    x_copy(2).start()
    w_copy(0).start()
    w_copy(2).start()

    def bcast_keys(jds):
        for jd in jds:
            col = jnp.broadcast_to(kv_ref[:, :, jd:jd + 1], kv_ref.shape)
            kb_ref[jd] = _unpack(col).astype(f32)

    def ln_block(b):
        xn = _layernorm(x_ref[NV + b * MR:NV + (b + 1) * MR, :].astype(f32))
        xu = _pack(xn)
        for cc in range(2):
            r0 = (2 * b + cc) * (CK // 2) + VK // 2
            xn_ref[r0:r0 + MK // 2, :] = xu[cc * (MK // 2):(cc + 1) * (MK // 2)]

    def k_proj(b):
        xu = jnp.concatenate(
            [xn_ref[(2 * b + cc) * (CK // 2) + VK // 2:(2 * b + cc + 1) * (CK // 2), :]
             for cc in range(2)], axis=0)
        k = jnp.dot(_unpack(xu), wqkv_ref[:, D:2 * D], preferred_element_type=f32)
        for g in range(NG):
            kp_ref[g, b * MK:(b + 1) * MK, :] = _pack(k[:, g * 128:(g + 1) * 128])

    early = 4
    jds = [j * DH + d for d in range(early) for j in range(HG)]

    x_copy(0).wait()
    xu0 = _pack(_layernorm(x_ref[0:NV, :].astype(f32)))
    for c in range(NC):
        xn_ref[c * (CK // 2):c * (CK // 2) + VK // 2, :] = xu0[c * 8:(c + 1) * 8]
    w_copy(1).wait()
    kv = jnp.dot(_unpack(xu0), wqkv_ref[:, D:2 * D], preferred_element_type=f32)
    for g in range(NG):
        kv_ref[g] = _pack(kv[:, g * 128:(g + 1) * 128])
    bcast_keys(jds[:3])
    x_copy(1).wait()
    for b in range(HP):
        ln_block(b)
    bcast_keys(jds[3:16])
    for b in range(HP - 1):
        k_proj(b)
    x_copy(2).wait()
    w_copy(0).wait()
    w_copy(2).wait()
    for n in range(3, 8):
        w_copy(n).start()
    for b in range(HP, NP):
        ln_block(b)
    wt_ref[0:D, :] = wqkv_ref[:, 0:D].astype(f32).T.astype(bf16)
    wt_ref[D:2 * D, :] = wqkv_ref[:, 2 * D:3 * D].astype(f32).T.astype(bf16)
    bcast_keys(jds[16:])
    for b in range(HP - 1, NP):
        k_proj(b)
    qscale = (DH ** -0.5) * math.log2(math.e)
    for b in range(NP):
        bcast_keys([b * DH + d for d in range(early, DH)])
        xp = _unpack(xn_ref[b * (TP // 2):(b + 1) * (TP // 2), :])
        qv = lax.dot_general(wt_ref[...], xp, (((1,), (1,)), ((), ())),
                             preferred_element_type=f32)
        qp_ref[:, b * TP:(b + 1) * TP] = _pack(qv[0:D] * qscale)
        vp_ref[:, b * TP:(b + 1) * TP] = _pack(qv[D:2 * D])

    NI = NQ * NG

    def unit_index(i, j):
        h = (i % NG) * HG + j
        return h, pl.multiple_of(h * 8, 8), pl.ds(pl.multiple_of((i // NG) * TQ, TQ), TQ)

    def stage_q(i, j, lo, hi):
        _, h8, cols = unit_index(i, j)
        qf = _unpack(qp_ref[pl.ds(h8, 8), cols]).astype(f32)
        for d in range(lo, hi):
            qs_refs[j][d] = jnp.broadcast_to(qf[d:d + 1, :], (8, TQ))

    def pv_step(i, j, c, row0, acc, inv_l, link=None):
        _, h8, cols = unit_index(i, j)
        vt = _unpack(vp_ref[pl.ds(h8, 8), c * CK:(c + 1) * CK])
        d = jnp.dot(vt, _unpack(pt_refs[c % RING][pl.ds(row0, CK // 2), :]),
                    preferred_element_type=f32)
        if acc is None:
            acc = jnp.where(link[0], link[1], d)
        else:
            acc = acc + d
        if c == NC - 1:
            op_ref[pl.ds(h8, 8), cols] = _pack(acc * jnp.concatenate([inv_l, inv_l], axis=0))
        return acc

    def inv_denominator(i, j, l8):
        h, _, cols = unit_index(i, j)
        l = jnp.sum(l8, axis=0, keepdims=True)
        l_ref[pl.ds(h, 1), cols] = l
        inv = pl.reciprocal(l, approx=True)
        inv = inv * (2.0 - l * inv)
        return jnp.broadcast_to(inv, l8.shape)

    def fast_group(i, carry):
        z1 = lax.shift_right_logical(i, 20)
        row0 = pl.multiple_of(z1 * 8, 8)
        never = lax.broadcasted_iota(i32, (VK, 128), 0) < z1
        never_wide = lax.broadcasted_iota(i32, (DH, TQ), 0) < z1
        g = i % NG
        grp = {j: i for j in range(HG)}
        grp[-1] = (i + NI - 1) % NI
        grp[HG] = jnp.minimum(i + 1, NI - 1)
        acc = {-1: carry[0]}
        l8 = {-1: carry[1]}
        pend = [(-1, c) for c in range(NC - LAG, NC)]
        prev = None
        for j in range(HG):
            _, h8, cols = unit_index(i, j)
            qrow = qp_ref[pl.ds(h8, 8), cols]
            z = jnp.zeros_like(qrow)
            w = _unpack(jnp.concatenate([qrow if b == j else z for b in range(HG)], axis=0))
            acc[j] = None
            l8[j] = None
            jn = (j + 1) % HG
            for c in range(NC):
                pt_ref = pt_refs[c % RING]
                base = c * (MK // 2)
                kc = _unpack(jnp.concatenate(
                    [kp_ref[g, base + b * 8:base + (b + 1) * 8, :] for b in range(6, -1, -1)],
                    axis=0))
                p = jnp.exp2(jnp.dot(kc, w, preferred_element_type=f32))
                cl = jnp.sum(p.reshape(MK // 8, 8, TQ), axis=0)
                l8[j] = cl if l8[j] is None else l8[j] + cl
                for b in range(7):
                    pt_ref[(7 - b) * 8:(8 - b) * 8, :] = _pack(p[b * 16:(b + 1) * 16, :])
                pend.append((j, c))
                pj, pc = pend.pop(0)
                link = (never_wide, acc[pj - 1]) if pc == 0 else None
                acc[pj] = pv_step(grp[pj], pj % HG, pc, row0, acc[pj], l8[pj], link)

                tie = None
                if c in (7, 9, 11, 13):
                    tie = qs_refs[jn][z1, :, 0:128]
                    tie = jnp.concatenate([tie, tie], axis=0)
                tiles = []
                for t in range(TQ // 128):
                    a = None
                    for d0 in range(0, DH, 4):
                        kb = kb_ref[pl.ds(j * DH + d0 + z1, 4), g, c * VK:(c + 1) * VK, :]
                        qd = qs_refs[j][pl.ds(z1 + d0, 4), :, t * 128:(t + 1) * 128]
                        pr = kb * jnp.concatenate([qd, qd], axis=1)
                        if d0 > 0:
                            a = jnp.sum(jnp.concatenate([a[None], pr], axis=0), axis=0)
                            continue
                        a = pr[0]
                        if t == 0 and tie is not None:
                            a = jnp.where(never, tie, a)
                        a = a + pr[1] + pr[2]
                        if prev is not None:
                            a = jnp.where(never, prev, a)
                        a = a + pr[3]
                    prev = a
                    tiles.append(a)
                p = jnp.exp2(jnp.concatenate(tiles, axis=1))
                l8[j] = l8[j] + (p[0:8] + p[8:16])
                pt_ref[0:8, :] = _pack(p)
                if c == NC - 1:
                    l8[j] = inv_denominator(i, j, l8[j])
                if c in (6, 8, 10, 12):
                    stage_q(grp[j + 1], jn, (c - 6) * 2, (c - 6) * 2 + 4)
        return acc[HG - 1], l8[HG - 1]

    stage_q(0, 0, 0, DH)
    for c in range(NC - LAG, NC):
        pt_refs[c % RING][...] = jnp.zeros((CK // 2, TQ), u32)
    acc, inv_l = lax.fori_loop(0, NI, fast_group,
                               (jnp.zeros((DH, TQ), f32), jnp.ones((8, TQ), f32)))
    for c in range(NC - LAG, NC):
        acc = pv_step(NI - 1, HG - 1, c, 0, acc, inv_l)

    l_all = l_ref[...]
    safe = jnp.logical_and(jnp.min(l_all) >= L_LO, jnp.max(l_all) <= L_HI)

    @pl.when(jnp.logical_not(safe))
    def _():
        def unit(u, carry):
            h = u % H
            g = h // HG
            j = h % HG
            cols = pl.ds(pl.multiple_of((u // H) * TQ, TQ), TQ)
            h8 = pl.multiple_of(h * 8, 8)
            qrow = qp_ref[pl.ds(h8, 8), cols]
            z = jnp.zeros_like(qrow)
            w = _unpack(jnp.concatenate(
                [jnp.where(j == b, qrow, z) for b in range(HG)], axis=0))

            def scores(c):
                kc = jnp.concatenate(
                    [kv_ref[g, pl.ds(pl.multiple_of(c * 8, 8), 8), :],
                     kp_ref[g, pl.ds(pl.multiple_of(c * (MK // 2), 8), MK // 2), :]], axis=0)
                return jnp.dot(_unpack(kc), w, preferred_element_type=f32)

            def max_body(c, m):
                return jnp.maximum(m, jnp.max(scores(c), axis=0, keepdims=True))

            m = lax.fori_loop(0, NC, max_body, jnp.full((1, TQ), -jnp.inf, f32))

            def sum_body(c, la):
                l, a = la
                p = jnp.exp2(scores(c) - m)
                vt = _unpack(vp_ref[pl.ds(h8, 8), pl.ds(pl.multiple_of(c * CK, CK), CK)])
                a = a + jnp.dot(vt, p.astype(bf16), preferred_element_type=f32)
                return l + jnp.sum(p, axis=0, keepdims=True), a

            l, a = lax.fori_loop(0, NC, sum_body,
                                 (jnp.zeros((1, TQ), f32), jnp.zeros((DH, TQ), f32)))
            op_ref[pl.ds(h8, 8), cols] = _pack(a * (1.0 / l))
            return carry

        lax.fori_loop(0, NQ * H, unit, 0)

    def out_copy(n):
        rows = pl.ds(0, NV) if n == NP else pl.ds(NV + n * MR, MR)
        return pltpu.make_async_copy(o_ref.at[rows, :], o_hbm.at[rows, :], osem.at[n])

    send_after = {7: range(0, 4), 13: range(4, 7), 15: range(7, NP + 1)}

    def token_spans(c):
        return ((0, c * VK, VK), (VK, NV + c * MK, MK))

    w_copy(3).wait()
    w_copy(7).wait()
    wr = jnp.broadcast_to(wr_ref[pl.ds(0, D)].astype(f32).reshape(1, D), (16, D)).astype(bf16)
    wo = wo_ref[...]

    def out_proj(c):
        ot = _unpack(op_ref[:, c * CK:(c + 1) * CK])
        return lax.dot_general(ot, wo, (((0,), (0,)), ((), ())),
                               preferred_element_type=f32)

    def residual_ln(c, attn):
        xb = jnp.concatenate(
            [x_ref[t0:t0 + n, :].astype(f32) for _, t0, n in token_spans(c)], axis=0)
        h = _rb(xb + attn)
        hn = _layernorm_bf16(h).astype(bf16)
        hnf = hn.astype(f32)
        o = h + hnf
        for p0, t0, n in token_spans(c):
            h_ref[t0:t0 + n, :] = h[p0:p0 + n]
            hn_ref[t0:t0 + n, :] = hnf[p0:p0 + n]
            o_ref[t0:t0 + n, :] = o[p0:p0 + n].astype(bf16)
        for n in send_after.get(c, ()):
            out_copy(n).start()
        return hn

    def router(c, hn):
        r = lax.dot_general(wr, hn, (((1,), (1,)), ((), ())), preferred_element_type=f32)
        r = jnp.clip(_rb(r[0:8, :]), -BF16_MAX, BF16_MAX)
        r = jnp.where(jnp.abs(r) < F32_TINY, F32_TINY, r)
        off = lax.broadcasted_iota(i32, r.shape, 1)
        tok = off + jnp.where(off < VK, c * VK, NV + c * MK - VK)
        key = pltpu.bitcast(r, i32) | jnp.where(r < 0, tok, S - 1 - tok)
        return pltpu.bitcast(key, f32)

    attn = out_proj(0)
    hn_prev = None
    keys = []
    for c in range(NC):
        attn_next = out_proj(c + 1) if c + 1 < NC else None
        if hn_prev is not None:
            keys.append(router(c - 1, hn_prev))
        hn_prev = residual_ln(c, attn)
        attn = attn_next
    keys.append(router(NC - 1, hn_prev))

    top, sec = keys[0], jnp.full(keys[0].shape, -jnp.inf, f32)
    for k in keys[1:]:
        sec = jnp.maximum(sec, jnp.minimum(top, k))
        top = jnp.maximum(top, k)
    k1 = jnp.max(top, axis=1, keepdims=True)
    k2 = jnp.max(jnp.where(top == k1, sec, top), axis=1, keepdims=True)

    def decode(k):
        bits = pltpu.bitcast(jnp.broadcast_to(k, (8, 128)), i32)
        low = bits & 0xFFFF
        tok = jnp.where(bits < 0, low, S - 1 - low)
        score = pltpu.bitcast(bits & jnp.int32(-65536), f32)
        return jnp.clip(tok[0, 0], 0, S - 1), score[0:1, 0:1]

    i1, r1 = decode(k1)
    i2, r2 = decode(k2)
    row16 = lax.broadcasted_iota(i32, (16, D), 0)
    first = row16 == 0
    hsel = jnp.where(first, h_ref[pl.ds(i1, 1), :], h_ref[pl.ds(i2, 1), :])
    xsel = jnp.where(first, hn_ref[pl.ds(i1, 1), :], hn_ref[pl.ds(i2, 1), :])
    xs = xsel.astype(bf16)
    w_copy(4).wait()
    w_copy(5).wait()
    w_copy(6).wait()
    gpre = _rb(jnp.dot(xs, wg_ref[...], preferred_element_type=f32))
    gate = _rb(gpre * jax.nn.sigmoid(gpre))
    up = _rb(jnp.dot(xs, wu_ref[...], preferred_element_type=f32))
    y = _rb(jnp.dot((gate * up).astype(bf16), wd_ref[...], preferred_element_type=f32))
    y = _rb(y * _rb(jax.nn.sigmoid(jnp.where(first, r1, r2))))
    osel = hsel + _rb(xsel + y)
    for n in range(NP + 1):
        out_copy(n).wait()
    bases = [pl.multiple_of(lax.shift_right_logical(idx, 4) * 16, 16) for idx in (i1, i2)]
    olds = [o_ref[pl.ds(base, 16), :].astype(f32) for base in bases]
    for base, old in zip(bases, olds):
        t = row16 + base
        new = jnp.where(t == i1, osel[0:1, :], jnp.where(t == i2, osel[1:2, :], old))
        o_ref[pl.ds(base, 16), :] = new.astype(bf16)
    patch = [pltpu.make_async_copy(o_ref.at[pl.ds(base, 16), :], o_hbm.at[pl.ds(base, 16), :],
                                   osem.at[n]) for n, base in enumerate(bases)]
    patch[0].start()

    @pl.when(bases[0] != bases[1])
    def _():
        patch[1].start()
        patch[1].wait()

    patch[0].wait()


@jax.jit
def pallas_sequential_preLN__mha_block__moe_arch_mod__prompt_kernel(
    A_x: jax.Array,
    A_wqkv: jax.Array,
    A_wo: jax.Array,
    B_x: jax.Array,
    B_w_r: jax.Array,
    B_w_gate: jax.Array,
    B_w_up: jax.Array,
    B_w_down: jax.Array,
):
    B, S, D = A_x.shape
    F = B_w_gate.shape[1]
    assert B == 1 and D == H * DH and S == 2048
    hbm = pl.BlockSpec(memory_space=pl.ANY)
    NC = S // CK
    NV = NC * VK
    out = pl.pallas_call(
        _kernel,
        out_shape=jax.ShapeDtypeStruct((S, D), A_x.dtype),
        in_specs=[hbm] * 7,
        out_specs=hbm,
        scratch_shapes=[
            pltpu.VMEM((S, D), bf16),
            pltpu.VMEM((S // 2, D), u32),
            pltpu.VMEM((D, 3 * D), bf16),
            pltpu.VMEM((2 * D, D), bf16),
            pltpu.VMEM((H // HG, NC * MK // 2, 128), u32),
            pltpu.VMEM((H // HG, NV // 2, 128), u32),
            pltpu.VMEM((128, H // HG, NV, 128), f32),
            pltpu.VMEM((D // 2, S), u32),
            pltpu.VMEM((D // 2, S), u32),
            pltpu.VMEM((D // 2, S), u32),
            pltpu.VMEM((H, S), f32),
            pltpu.VMEM((S, D), f32),
            pltpu.VMEM((S, D), f32),
            pltpu.VMEM((S, D), bf16),
            pltpu.VMEM((D, D), bf16),
            pltpu.VMEM((D, F), bf16),
            pltpu.VMEM((D, F), bf16),
            pltpu.VMEM((F, D), bf16),
            pltpu.VMEM((16 * D,), bf16),
            pltpu.SemaphoreType.DMA((3,)),
            pltpu.SemaphoreType.DMA((8,)),
            pltpu.SemaphoreType.DMA((S // TP + 1,)),
        ] + [pltpu.VMEM((CK // 2, TQ), u32)] * RING + [pltpu.VMEM((DH, 8, TQ), f32)] * HG,
        compiler_params=pltpu.CompilerParams(vmem_limit_bytes=120 * 1024 * 1024),
    )(A_x.reshape(S, D), A_wqkv, B_w_r, A_wo, B_w_gate, B_w_up, B_w_down)
    return out.reshape(B, S, D)
```

```python
import math

import jax
import jax.numpy as jnp
from jax import lax
import jax.experimental.pallas as pl
import jax.experimental.pallas.tpu as pltpu

f32, bf16, u32, i32 = jnp.float32, jnp.bfloat16, jnp.uint32, jnp.int32

H = 32
DH = 16
HG = 8
TQ = 512
CK = 128
VK = 16
MK = CK - VK
LAG = 4
RING = 8
TP = 2 * CK
EPS = 1e-5
BF16_MAX = 3.3895313892515355e38
F32_TINY = 2.0 ** -126
L_LO, L_HI = 2.0 ** -60, 2.0 ** 60


def _rb(x):
    return x.astype(bf16).astype(f32)


def _mean(x):
    return jnp.sum(x, axis=-1, keepdims=True) * (1.0 / x.shape[-1])


def _layernorm(x):
    xc = x - _mean(x)
    return xc * lax.rsqrt(_mean(xc * xc) + EPS)


def _layernorm_bf16(x):
    mean = _mean(x)
    xc = x - mean
    v = _rb(_rb(_mean(xc * xc)) + EPS)
    den = _rb(v * lax.rsqrt(v))
    inv = pl.reciprocal(den, approx=True)
    inv = inv * (2.0 - den * inv)
    return (x - _rb(mean)) * inv


def _pack(x):
    return pltpu.bitcast(x.astype(bf16), u32)


def _unpack(x):
    return pltpu.bitcast(x, bf16)


def _kernel(x_hbm, wqkv_hbm, wr_hbm, wo_hbm, wg_hbm, wu_hbm, wd_hbm, o_hbm,
            x_ref, xn_ref, wqkv_ref, wt_ref, kp_ref, kv_ref, kb_ref, qp_ref, vp_ref, op_ref,
            l_ref, h_ref, hn_ref, o_ref, wo_ref, wg_ref, wu_ref, wd_ref, wr_ref,
            xsem, wsem, osem, *stage):
    pt_refs = stage[:RING]
    qs_refs = stage[RING:]
    S, D = x_ref.shape
    NQ = S // TQ
    NC = S // CK
    NG = H // HG
    NP = S // TP
    HP = NP // 2
    NV = NC * VK
    MR = 2 * MK

    def x_copy(n):
        rows = pl.ds(0, NV) if n == 0 else pl.ds(NV + (n - 1) * HP * MR, HP * MR)
        return pltpu.make_async_copy(x_hbm.at[rows, :], x_ref.at[rows, :], xsem.at[n])

    def w_copy(n):
        if n < 3:
            cols = pl.ds(n * D, D)
            return pltpu.make_async_copy(wqkv_hbm.at[:, cols], wqkv_ref.at[:, cols], wsem.at[n])
        src, dst = ((wo_hbm, wo_ref), (wg_hbm, wg_ref), (wu_hbm, wu_ref), (wd_hbm, wd_ref),
                    (wr_hbm, wr_ref.at[pl.ds(0, D)]))[n - 3]
        return pltpu.make_async_copy(src, dst, wsem.at[n])

    x_copy(0).start()
    w_copy(1).start()
    x_copy(1).start()
    x_copy(2).start()
    w_copy(0).start()
    w_copy(2).start()

    def bcast_keys(jds):
        for jd in jds:
            col = jnp.broadcast_to(kv_ref[:, :, jd:jd + 1], kv_ref.shape)
            kb_ref[jd] = _unpack(col).astype(f32)

    def ln_block(b):
        xn = _layernorm(x_ref[NV + b * MR:NV + (b + 1) * MR, :].astype(f32))
        xu = _pack(xn)
        for cc in range(2):
            r0 = (2 * b + cc) * (CK // 2) + VK // 2
            xn_ref[r0:r0 + MK // 2, :] = xu[cc * (MK // 2):(cc + 1) * (MK // 2)]

    def k_proj(b):
        xu = jnp.concatenate(
            [xn_ref[(2 * b + cc) * (CK // 2) + VK // 2:(2 * b + cc + 1) * (CK // 2), :]
             for cc in range(2)], axis=0)
        k = jnp.dot(_unpack(xu), wqkv_ref[:, D:2 * D], preferred_element_type=f32)
        for g in range(NG):
            kp_ref[g, b * MK:(b + 1) * MK, :] = _pack(k[:, g * 128:(g + 1) * 128])

    early = 4
    jds = [j * DH + d for d in range(early) for j in range(HG)]

    x_copy(0).wait()
    xu0 = _pack(_layernorm(x_ref[0:NV, :].astype(f32)))
    for c in range(NC):
        xn_ref[c * (CK // 2):c * (CK // 2) + VK // 2, :] = xu0[c * 8:(c + 1) * 8]
    w_copy(1).wait()
    kv = jnp.dot(_unpack(xu0), wqkv_ref[:, D:2 * D], preferred_element_type=f32)
    for g in range(NG):
        kv_ref[g] = _pack(kv[:, g * 128:(g + 1) * 128])
    bcast_keys(jds[:3])
    x_copy(1).wait()
    for b in range(HP):
        ln_block(b)
    bcast_keys(jds[3:16])
    for b in range(HP - 1):
        k_proj(b)
    x_copy(2).wait()
    w_copy(0).wait()
    w_copy(2).wait()
    for n in range(3, 8):
        w_copy(n).start()
    for b in range(HP, NP):
        ln_block(b)
    wt_ref[0:D, :] = wqkv_ref[:, 0:D].astype(f32).T.astype(bf16)
    wt_ref[D:2 * D, :] = wqkv_ref[:, 2 * D:3 * D].astype(f32).T.astype(bf16)
    bcast_keys(jds[16:])
    for b in range(HP - 1, NP):
        k_proj(b)
    qscale = (DH ** -0.5) * math.log2(math.e)
    for b in range(NP):
        bcast_keys([b * DH + d for d in range(early, DH)])
        xp = _unpack(xn_ref[b * (TP // 2):(b + 1) * (TP // 2), :])
        qv = lax.dot_general(wt_ref[...], xp, (((1,), (1,)), ((), ())),
                             preferred_element_type=f32)
        qp_ref[:, b * TP:(b + 1) * TP] = _pack(qv[0:D] * qscale)
        vp_ref[:, b * TP:(b + 1) * TP] = _pack(qv[D:2 * D])

    NI = NQ * NG

    def unit_index(i, j):
        h = (i % NG) * HG + j
        return h, pl.multiple_of(h * 8, 8), pl.ds(pl.multiple_of((i // NG) * TQ, TQ), TQ)

    def stage_q(unit, j, lo, hi):
        _, h8, cols = unit
        qf = _unpack(qp_ref[pl.ds(h8, 8), cols]).astype(f32)
        for d in range(lo, hi):
            qs_refs[j][d] = jnp.broadcast_to(qf[d:d + 1, :], (8, TQ))

    def pv_step(unit, c, row0, acc, inv_l, link=None):
        _, h8, cols = unit
        vt = _unpack(vp_ref[pl.ds(h8, 8), c * CK:(c + 1) * CK])
        d = jnp.dot(vt, _unpack(pt_refs[c % RING][pl.ds(row0, CK // 2), :]),
                    preferred_element_type=f32)
        if acc is None:
            acc = jnp.where(link[0], link[1], d)
        else:
            acc = acc + d
        if c == NC - 1:
            op_ref[pl.ds(h8, 8), cols] = _pack(acc * jnp.concatenate([inv_l, inv_l], axis=0))
        return acc

    def inv_denominator(unit, l8):
        h, _, cols = unit
        l = jnp.sum(l8, axis=0, keepdims=True)
        l_ref[pl.ds(h, 1), cols] = l
        inv = pl.reciprocal(l, approx=True)
        inv = inv * (2.0 - l * inv)
        return jnp.broadcast_to(inv, l8.shape)

    def fast_group(i, carry):
        z1 = lax.shift_right_logical(i, 20)
        row0 = pl.multiple_of(z1 * 8, 8)
        never = lax.broadcasted_iota(i32, (VK, 128), 0) < z1
        never_wide = lax.broadcasted_iota(i32, (DH, TQ), 0) < z1
        g = i % NG
        units = {j: unit_index(i, j) for j in range(HG)}
        units[-1] = unit_index((i + NI - 1) % NI, HG - 1)
        units[HG] = unit_index(jnp.minimum(i + 1, NI - 1), 0)
        dims = [z1 + d0 for d0 in range(0, DH, 4)]
        acc = {-1: carry[0]}
        l8 = {-1: carry[1]}
        pend = [(-1, c) for c in range(NC - LAG, NC)]
        prev = None
        for j in range(HG):
            _, h8, cols = units[j]
            kdims = [d0 + j * DH for d0 in dims]
            qrow = qp_ref[pl.ds(h8, 8), cols]
            z = jnp.zeros_like(qrow)
            w = _unpack(jnp.concatenate([qrow if b == j else z for b in range(HG)], axis=0))
            acc[j] = None
            l8[j] = None
            jn = (j + 1) % HG
            for c in range(NC):
                pt_ref = pt_refs[c % RING]
                base = c * (MK // 2)
                kc = _unpack(jnp.concatenate(
                    [kp_ref[g, base + b * 8:base + (b + 1) * 8, :] for b in range(6, -1, -1)],
                    axis=0))
                p = jnp.exp2(jnp.dot(kc, w, preferred_element_type=f32))
                cl = jnp.sum(p.reshape(MK // 8, 8, TQ), axis=0)
                l8[j] = cl if l8[j] is None else l8[j] + cl
                for b in range(7):
                    pt_ref[(7 - b) * 8:(8 - b) * 8, :] = _pack(p[b * 16:(b + 1) * 16, :])
                pend.append((j, c))
                pj, pc = pend.pop(0)
                link = (never_wide, acc[pj - 1]) if pc == 0 else None
                acc[pj] = pv_step(units[pj], pc, row0, acc[pj], l8[pj], link)

                tie = None
                if c in (7, 9, 11, 13):
                    tie = qs_refs[jn][z1, :, 0:128]
                    tie = jnp.concatenate([tie, tie], axis=0)
                tiles = []
                for t in range(TQ // 128):
                    a = None
                    for d0, kd0 in zip(dims, kdims):
                        kb = kb_ref[pl.ds(kd0, 4), g, c * VK:(c + 1) * VK, :]
                        qd = qs_refs[j][pl.ds(d0, 4), :, t * 128:(t + 1) * 128]
                        pr = kb * jnp.concatenate([qd, qd], axis=1)
                        if a is not None:
                            a = jnp.sum(jnp.concatenate([a[None], pr], axis=0), axis=0)
                            continue
                        a = pr[0]
                        if t == 0 and tie is not None:
                            a = jnp.where(never, tie, a)
                        a = a + pr[1] + pr[2]
                        if prev is not None:
                            a = jnp.where(never, prev, a)
                        a = a + pr[3]
                    prev = a
                    tiles.append(a)
                p = jnp.exp2(jnp.concatenate(tiles, axis=1))
                l8[j] = l8[j] + (p[0:8] + p[8:16])
                pt_ref[0:8, :] = _pack(p)
                if c == NC - 1:
                    l8[j] = inv_denominator(units[j], l8[j])
                if c in (6, 8, 10, 12):
                    stage_q(units[j + 1], jn, (c - 6) * 2, (c - 6) * 2 + 4)
        return acc[HG - 1], l8[HG - 1]

    stage_q(unit_index(0, 0), 0, 0, DH)
    for c in range(NC - LAG, NC):
        pt_refs[c % RING][...] = jnp.zeros((CK // 2, TQ), u32)
    acc, inv_l = lax.fori_loop(0, NI, fast_group,
                               (jnp.zeros((DH, TQ), f32), jnp.ones((8, TQ), f32)))
    for c in range(NC - LAG, NC):
        acc = pv_step(unit_index(NI - 1, HG - 1), c, 0, acc, inv_l)

    l_all = l_ref[...]
    safe = jnp.logical_and(jnp.min(l_all) >= L_LO, jnp.max(l_all) <= L_HI)

    @pl.when(jnp.logical_not(safe))
    def _():
        def unit(u, carry):
            h = u % H
            g = h // HG
            j = h % HG
            cols = pl.ds(pl.multiple_of((u // H) * TQ, TQ), TQ)
            h8 = pl.multiple_of(h * 8, 8)
            qrow = qp_ref[pl.ds(h8, 8), cols]
            z = jnp.zeros_like(qrow)
            w = _unpack(jnp.concatenate(
                [jnp.where(j == b, qrow, z) for b in range(HG)], axis=0))

            def scores(c):
                kc = jnp.concatenate(
                    [kv_ref[g, pl.ds(pl.multiple_of(c * 8, 8), 8), :],
                     kp_ref[g, pl.ds(pl.multiple_of(c * (MK // 2), 8), MK // 2), :]], axis=0)
                return jnp.dot(_unpack(kc), w, preferred_element_type=f32)

            def max_body(c, m):
                return jnp.maximum(m, jnp.max(scores(c), axis=0, keepdims=True))

            m = lax.fori_loop(0, NC, max_body, jnp.full((1, TQ), -jnp.inf, f32))

            def sum_body(c, la):
                l, a = la
                p = jnp.exp2(scores(c) - m)
                vt = _unpack(vp_ref[pl.ds(h8, 8), pl.ds(pl.multiple_of(c * CK, CK), CK)])
                a = a + jnp.dot(vt, p.astype(bf16), preferred_element_type=f32)
                return l + jnp.sum(p, axis=0, keepdims=True), a

            l, a = lax.fori_loop(0, NC, sum_body,
                                 (jnp.zeros((1, TQ), f32), jnp.zeros((DH, TQ), f32)))
            op_ref[pl.ds(h8, 8), cols] = _pack(a * (1.0 / l))
            return carry

        lax.fori_loop(0, NQ * H, unit, 0)

    def out_copy(n):
        rows = pl.ds(0, NV) if n == NP else pl.ds(NV + n * MR, MR)
        return pltpu.make_async_copy(o_ref.at[rows, :], o_hbm.at[rows, :], osem.at[n])

    send_after = {7: range(0, 4), 13: range(4, 7), 15: range(7, NP + 1)}

    def token_spans(c):
        return ((0, c * VK, VK), (VK, NV + c * MK, MK))

    w_copy(3).wait()
    w_copy(7).wait()
    wr = jnp.broadcast_to(wr_ref[pl.ds(0, D)].astype(f32).reshape(1, D), (16, D)).astype(bf16)
    wo = wo_ref[...]

    def out_proj(c):
        ot = _unpack(op_ref[:, c * CK:(c + 1) * CK])
        return lax.dot_general(ot, wo, (((0,), (0,)), ((), ())),
                               preferred_element_type=f32)

    def residual_ln(c, attn):
        xb = jnp.concatenate(
            [x_ref[t0:t0 + n, :].astype(f32) for _, t0, n in token_spans(c)], axis=0)
        h = _rb(xb + attn)
        hn = _layernorm_bf16(h).astype(bf16)
        hnf = hn.astype(f32)
        o = h + hnf
        for p0, t0, n in token_spans(c):
            h_ref[t0:t0 + n, :] = h[p0:p0 + n]
            hn_ref[t0:t0 + n, :] = hnf[p0:p0 + n]
            o_ref[t0:t0 + n, :] = o[p0:p0 + n].astype(bf16)
        for n in send_after.get(c, ()):
            out_copy(n).start()
        return hn

    def router(c, hn):
        r = lax.dot_general(wr, hn, (((1,), (1,)), ((), ())), preferred_element_type=f32)
        r = jnp.clip(_rb(r[0:8, :]), -BF16_MAX, BF16_MAX)
        r = jnp.where(jnp.abs(r) < F32_TINY, F32_TINY, r)
        off = lax.broadcasted_iota(i32, r.shape, 1)
        tok = off + jnp.where(off < VK, c * VK, NV + c * MK - VK)
        key = pltpu.bitcast(r, i32) | jnp.where(r < 0, tok, S - 1 - tok)
        return pltpu.bitcast(key, f32)

    attn = out_proj(0)
    hn_prev = None
    keys = []
    for c in range(NC):
        attn_next = out_proj(c + 1) if c + 1 < NC else None
        if hn_prev is not None:
            keys.append(router(c - 1, hn_prev))
        hn_prev = residual_ln(c, attn)
        attn = attn_next
    keys.append(router(NC - 1, hn_prev))

    top, sec = keys[0], jnp.full(keys[0].shape, -jnp.inf, f32)
    for k in keys[1:]:
        sec = jnp.maximum(sec, jnp.minimum(top, k))
        top = jnp.maximum(top, k)
    k1 = jnp.max(top, axis=1, keepdims=True)
    k2 = jnp.max(jnp.where(top == k1, sec, top), axis=1, keepdims=True)

    def decode(k):
        bits = pltpu.bitcast(jnp.broadcast_to(k, (8, 128)), i32)
        low = bits & 0xFFFF
        tok = jnp.where(bits < 0, low, S - 1 - low)
        score = pltpu.bitcast(bits & jnp.int32(-65536), f32)
        return jnp.clip(tok[0, 0], 0, S - 1), score[0:1, 0:1]

    i1, r1 = decode(k1)
    i2, r2 = decode(k2)
    row16 = lax.broadcasted_iota(i32, (16, D), 0)
    first = row16 == 0
    hsel = jnp.where(first, h_ref[pl.ds(i1, 1), :], h_ref[pl.ds(i2, 1), :])
    xsel = jnp.where(first, hn_ref[pl.ds(i1, 1), :], hn_ref[pl.ds(i2, 1), :])
    xs = xsel.astype(bf16)
    w_copy(4).wait()
    w_copy(5).wait()
    w_copy(6).wait()
    gpre = _rb(jnp.dot(xs, wg_ref[...], preferred_element_type=f32))
    gate = _rb(gpre * jax.nn.sigmoid(gpre))
    up = _rb(jnp.dot(xs, wu_ref[...], preferred_element_type=f32))
    y = _rb(jnp.dot((gate * up).astype(bf16), wd_ref[...], preferred_element_type=f32))
    y = _rb(y * _rb(jax.nn.sigmoid(jnp.where(first, r1, r2))))
    osel = hsel + _rb(xsel + y)
    for n in range(NP + 1):
        out_copy(n).wait()
    bases = [pl.multiple_of(lax.shift_right_logical(idx, 4) * 16, 16) for idx in (i1, i2)]
    olds = [o_ref[pl.ds(base, 16), :].astype(f32) for base in bases]
    for base, old in zip(bases, olds):
        t = row16 + base
        new = jnp.where(t == i1, osel[0:1, :], jnp.where(t == i2, osel[1:2, :], old))
        o_ref[pl.ds(base, 16), :] = new.astype(bf16)
    patch = [pltpu.make_async_copy(o_ref.at[pl.ds(base, 16), :], o_hbm.at[pl.ds(base, 16), :],
                                   osem.at[n]) for n, base in enumerate(bases)]
    patch[0].start()

    @pl.when(bases[0] != bases[1])
    def _():
        patch[1].start()
        patch[1].wait()

    patch[0].wait()


@jax.jit
def pallas_sequential_preLN__mha_block__moe_arch_mod__prompt_kernel(
    A_x: jax.Array,
    A_wqkv: jax.Array,
    A_wo: jax.Array,
    B_x: jax.Array,
    B_w_r: jax.Array,
    B_w_gate: jax.Array,
    B_w_up: jax.Array,
    B_w_down: jax.Array,
):
    B, S, D = A_x.shape
    F = B_w_gate.shape[1]
    assert B == 1 and D == H * DH and S == 2048
    hbm = pl.BlockSpec(memory_space=pl.ANY)
    NC = S // CK
    NV = NC * VK
    out = pl.pallas_call(
        _kernel,
        out_shape=jax.ShapeDtypeStruct((S, D), A_x.dtype),
        in_specs=[hbm] * 7,
        out_specs=hbm,
        scratch_shapes=[
            pltpu.VMEM((S, D), bf16),
            pltpu.VMEM((S // 2, D), u32),
            pltpu.VMEM((D, 3 * D), bf16),
            pltpu.VMEM((2 * D, D), bf16),
            pltpu.VMEM((H // HG, NC * MK // 2, 128), u32),
            pltpu.VMEM((H // HG, NV // 2, 128), u32),
            pltpu.VMEM((128, H // HG, NV, 128), f32),
            pltpu.VMEM((D // 2, S), u32),
            pltpu.VMEM((D // 2, S), u32),
            pltpu.VMEM((D // 2, S), u32),
            pltpu.VMEM((H, S), f32),
            pltpu.VMEM((S, D), f32),
            pltpu.VMEM((S, D), f32),
            pltpu.VMEM((S, D), bf16),
            pltpu.VMEM((D, D), bf16),
            pltpu.VMEM((D, F), bf16),
            pltpu.VMEM((D, F), bf16),
            pltpu.VMEM((F, D), bf16),
            pltpu.VMEM((16 * D,), bf16),
            pltpu.SemaphoreType.DMA((3,)),
            pltpu.SemaphoreType.DMA((8,)),
            pltpu.SemaphoreType.DMA((S // TP + 1,)),
        ] + [pltpu.VMEM((CK // 2, TQ), u32)] * RING + [pltpu.VMEM((DH, 8, TQ), f32)] * HG,
        compiler_params=pltpu.CompilerParams(vmem_limit_bytes=120 * 1024 * 1024),
    )(A_x.reshape(S, D), A_wqkv, B_w_r, A_wo, B_w_gate, B_w_up, B_w_down)
    return out.reshape(B, S, D)
```

```python
import math

import jax
import jax.numpy as jnp
from jax import lax
import jax.experimental.pallas as pl
import jax.experimental.pallas.tpu as pltpu

f32, bf16, u32, i32 = jnp.float32, jnp.bfloat16, jnp.uint32, jnp.int32

H = 32
DH = 16
HG = 8
TQ = 512
CK = 128
VK = 16
MK = CK - VK
LAG = 4
RING = 8
TP = 2 * CK
EPS = 1e-5
BF16_MAX = 3.3895313892515355e38
F32_TINY = 2.0 ** -126
L_LO, L_HI = 2.0 ** -60, 2.0 ** 60


def _rb(x):
    return x.astype(bf16).astype(f32)


def _mean(x):
    return jnp.sum(x, axis=-1, keepdims=True) * (1.0 / x.shape[-1])


def _layernorm(x):
    xc = x - _mean(x)
    return xc * lax.rsqrt(_mean(xc * xc) + EPS)


def _layernorm_bf16(x):
    mean = _mean(x)
    xc = x - mean
    v = _rb(_rb(_mean(xc * xc)) + EPS)
    den = _rb(v * lax.rsqrt(v))
    inv = pl.reciprocal(den, approx=True)
    inv = inv * (2.0 - den * inv)
    return (x - _rb(mean)) * inv


def _pack(x):
    return pltpu.bitcast(x.astype(bf16), u32)


def _unpack(x):
    return pltpu.bitcast(x, bf16)


def _kernel(x_hbm, wqkv_hbm, wr_hbm, wo_hbm, wg_hbm, wu_hbm, wd_hbm, o_hbm,
            x_ref, xn_ref, wqkv_ref, wt_ref, kp_ref, kv_ref, kb_ref, qp_ref, vp_ref, op_ref,
            l_ref, h_ref, hn_ref, o_ref, wo_ref, wg_ref, wu_ref, wd_ref, wr_ref,
            xsem, wsem, osem, *stage):
    pt_refs = stage[:RING]
    qs_refs = stage[RING:]
    S, D = x_ref.shape
    NQ = S // TQ
    NC = S // CK
    NG = H // HG
    NP = S // TP
    HP = NP // 2
    NV = NC * VK
    MR = 2 * MK

    def x_copy(n):
        rows = pl.ds(0, NV) if n == 0 else pl.ds(NV + (n - 1) * HP * MR, HP * MR)
        return pltpu.make_async_copy(x_hbm.at[rows, :], x_ref.at[rows, :], xsem.at[n])

    def w_copy(n):
        if n < 3:
            cols = pl.ds(n * D, D)
            return pltpu.make_async_copy(wqkv_hbm.at[:, cols], wqkv_ref.at[:, cols], wsem.at[n])
        src, dst = ((wo_hbm, wo_ref), (wg_hbm, wg_ref), (wu_hbm, wu_ref), (wd_hbm, wd_ref),
                    (wr_hbm, wr_ref.at[pl.ds(0, D)]))[n - 3]
        return pltpu.make_async_copy(src, dst, wsem.at[n])

    x_copy(0).start()
    w_copy(1).start()
    x_copy(1).start()
    x_copy(2).start()
    w_copy(0).start()
    w_copy(2).start()

    def bcast_keys(jds):
        for jd in jds:
            col = jnp.broadcast_to(kv_ref[:, :, jd:jd + 1], kv_ref.shape)
            kb_ref[jd] = _unpack(col).astype(f32)

    def ln_block(b):
        xn = _layernorm(x_ref[NV + b * MR:NV + (b + 1) * MR, :].astype(f32))
        xu = _pack(xn)
        for cc in range(2):
            r0 = (2 * b + cc) * (CK // 2) + VK // 2
            xn_ref[r0:r0 + MK // 2, :] = xu[cc * (MK // 2):(cc + 1) * (MK // 2)]

    def k_proj(b):
        xu = jnp.concatenate(
            [xn_ref[(2 * b + cc) * (CK // 2) + VK // 2:(2 * b + cc + 1) * (CK // 2), :]
             for cc in range(2)], axis=0)
        k = jnp.dot(_unpack(xu), wqkv_ref[:, D:2 * D], preferred_element_type=f32)
        for g in range(NG):
            kp_ref[g, b * MK:(b + 1) * MK, :] = _pack(k[:, g * 128:(g + 1) * 128])

    early = 4
    jds = [j * DH + d for d in range(early) for j in range(HG)]

    x_copy(0).wait()
    xu0 = _pack(_layernorm(x_ref[0:NV, :].astype(f32)))
    for c in range(NC):
        xn_ref[c * (CK // 2):c * (CK // 2) + VK // 2, :] = xu0[c * 8:(c + 1) * 8]
    w_copy(1).wait()
    kv = jnp.dot(_unpack(xu0), wqkv_ref[:, D:2 * D], preferred_element_type=f32)
    for g in range(NG):
        kv_ref[g] = _pack(kv[:, g * 128:(g + 1) * 128])
    bcast_keys(jds[:3])
    x_copy(1).wait()
    for b in range(HP):
        ln_block(b)
    bcast_keys(jds[3:16])
    for b in range(HP - 1):
        k_proj(b)
    x_copy(2).wait()
    w_copy(0).wait()
    w_copy(2).wait()
    for n in range(3, 8):
        w_copy(n).start()
    for b in range(HP, NP):
        ln_block(b)
    wt_ref[0:D, :] = wqkv_ref[:, 0:D].astype(f32).T.astype(bf16)
    wt_ref[D:2 * D, :] = wqkv_ref[:, 2 * D:3 * D].astype(f32).T.astype(bf16)
    bcast_keys(jds[16:])
    for b in range(HP - 1, NP):
        k_proj(b)
    qscale = (DH ** -0.5) * math.log2(math.e)
    for b in range(NP):
        bcast_keys([b * DH + d for d in range(early, DH)])
        xp = _unpack(xn_ref[b * (TP // 2):(b + 1) * (TP // 2), :])
        qv = lax.dot_general(wt_ref[...], xp, (((1,), (1,)), ((), ())),
                             preferred_element_type=f32)
        qp_ref[:, b * TP:(b + 1) * TP] = _pack(qv[0:D] * qscale)
        vp_ref[:, b * TP:(b + 1) * TP] = _pack(qv[D:2 * D])

    NI = NQ * NG

    def unit_index(i, j):
        h = (i % NG) * HG + j
        return h, pl.multiple_of(h * 8, 8), pl.ds(pl.multiple_of((i // NG) * TQ, TQ), TQ)

    def stage_q(unit, j, lo, hi):
        _, h8, cols = unit
        qf = _unpack(qp_ref[pl.ds(h8, 8), cols]).astype(f32)
        for d in range(lo, hi):
            qs_refs[j][d] = jnp.broadcast_to(qf[d:d + 1, :], (8, TQ))

    def pv_step(unit, c, row0, acc, inv_l, link=None):
        _, h8, cols = unit
        vt = _unpack(vp_ref[pl.ds(h8, 8), c * CK:(c + 1) * CK])
        d = jnp.dot(vt, _unpack(pt_refs[c % RING][pl.ds(row0, CK // 2), :]),
                    preferred_element_type=f32)
        if acc is None:
            acc = jnp.where(link[0], link[1], d)
        else:
            acc = acc + d
        if c == NC - 1:
            op_ref[pl.ds(h8, 8), cols] = _pack(acc * jnp.concatenate([inv_l, inv_l], axis=0))
        return acc

    def inv_denominator(unit, l8):
        h, _, cols = unit
        l = jnp.sum(l8, axis=0, keepdims=True)
        l_ref[pl.ds(h, 1), cols] = l
        inv = pl.reciprocal(l, approx=True)
        inv = inv * (2.0 - l * inv)
        return jnp.broadcast_to(inv, l8.shape)

    def fast_group(i, carry):
        z1 = lax.shift_right_logical(i, 20)
        row0 = pl.multiple_of(z1 * 8, 8)
        never = lax.broadcasted_iota(i32, (VK, 128), 0) < z1
        never_wide = lax.broadcasted_iota(i32, (DH, TQ), 0) < z1
        g = i % NG
        units = {j: unit_index(i, j) for j in range(HG)}
        units[-1] = unit_index((i + NI - 1) % NI, HG - 1)
        units[HG] = unit_index(jnp.minimum(i + 1, NI - 1), 0)
        dims = [z1 + d0 for d0 in range(0, DH, 4)]
        acc = {-1: carry[0]}
        l8 = {-1: carry[1]}
        pend = [(-1, c) for c in range(NC - LAG, NC)]
        prev = None
        for j in range(HG):
            _, h8, cols = units[j]
            kdims = [d0 + j * DH for d0 in dims]
            qrow = qp_ref[pl.ds(h8, 8), cols]
            z = jnp.zeros_like(qrow)
            w = _unpack(jnp.concatenate([qrow if b == j else z for b in range(HG)], axis=0))
            acc[j] = None
            l8[j] = None
            jn = (j + 1) % HG
            for c in range(NC):
                pt_ref = pt_refs[c % RING]
                base = c * (MK // 2)
                kc = _unpack(jnp.concatenate(
                    [kp_ref[g, base + b * 8:base + (b + 1) * 8, :] for b in range(6, -1, -1)],
                    axis=0))
                p = jnp.exp2(jnp.dot(kc, w, preferred_element_type=f32))
                cl = jnp.sum(p.reshape(MK // 8, 8, TQ), axis=0)
                l8[j] = cl if l8[j] is None else l8[j] + cl
                for b in range(7):
                    pt_ref[(7 - b) * 8:(8 - b) * 8, :] = _pack(p[b * 16:(b + 1) * 16, :])
                pend.append((j, c))
                pj, pc = pend.pop(0)
                link = (never_wide, acc[pj - 1]) if pc == 0 else None
                acc[pj] = pv_step(units[pj], pc, row0, acc[pj], l8[pj], link)

                tie = None
                if c in (7, 9, 11, 13):
                    tie = qs_refs[jn][z1, :, 0:128]
                    tie = jnp.concatenate([tie, tie], axis=0)
                tiles = []
                for t in range(TQ // 128):
                    a = None
                    for d0, kd0 in zip(dims, kdims):
                        kb = kb_ref[pl.ds(kd0, 4), g, c * VK:(c + 1) * VK, :]
                        qd = qs_refs[j][pl.ds(d0, 4), :, t * 128:(t + 1) * 128]
                        pr = kb * jnp.concatenate([qd, qd], axis=1)
                        if a is not None:
                            a = jnp.sum(jnp.concatenate([a[None], pr], axis=0), axis=0)
                            continue
                        a = pr[0]
                        if t == 0 and tie is not None:
                            a = jnp.where(never, tie, a)
                        a = a + pr[1] + pr[2]
                        if prev is not None:
                            a = jnp.where(never, prev, a)
                        a = a + pr[3]
                    prev = a
                    tiles.append(a)
                p = jnp.exp2(jnp.concatenate(tiles, axis=1))
                l8[j] = l8[j] + (p[0:8] + p[8:16])
                pt_ref[0:8, :] = _pack(p)
                if c == NC - 1:
                    l8[j] = inv_denominator(units[j], l8[j])
                if c in (6, 8, 10, 12):
                    stage_q(units[j + 1], jn, (c - 6) * 2, (c - 6) * 2 + 4)
        return acc[HG - 1], l8[HG - 1]

    stage_q(unit_index(0, 0), 0, 0, DH)
    for c in range(NC - LAG, NC):
        pt_refs[c % RING][...] = jnp.zeros((CK // 2, TQ), u32)
    acc, inv_l = lax.fori_loop(0, NI, fast_group,
                               (jnp.zeros((DH, TQ), f32), jnp.ones((8, TQ), f32)))
    for c in range(NC - LAG, NC):
        acc = pv_step(unit_index(NI - 1, HG - 1), c, 0, acc, inv_l)

    l_all = l_ref[...]
    safe = jnp.logical_and(jnp.min(l_all) >= L_LO, jnp.max(l_all) <= L_HI)

    @pl.when(jnp.logical_not(safe))
    def _():
        def unit(u, carry):
            h = u % H
            g = h // HG
            j = h % HG
            cols = pl.ds(pl.multiple_of((u // H) * TQ, TQ), TQ)
            h8 = pl.multiple_of(h * 8, 8)
            qrow = qp_ref[pl.ds(h8, 8), cols]
            z = jnp.zeros_like(qrow)
            w = _unpack(jnp.concatenate(
                [jnp.where(j == b, qrow, z) for b in range(HG)], axis=0))

            def scores(c):
                kc = jnp.concatenate(
                    [kv_ref[g, pl.ds(pl.multiple_of(c * 8, 8), 8), :],
                     kp_ref[g, pl.ds(pl.multiple_of(c * (MK // 2), 8), MK // 2), :]], axis=0)
                return jnp.dot(_unpack(kc), w, preferred_element_type=f32)

            def max_body(c, m):
                return jnp.maximum(m, jnp.max(scores(c), axis=0, keepdims=True))

            m = lax.fori_loop(0, NC, max_body, jnp.full((1, TQ), -jnp.inf, f32))

            def sum_body(c, la):
                l, a = la
                p = jnp.exp2(scores(c) - m)
                vt = _unpack(vp_ref[pl.ds(h8, 8), pl.ds(pl.multiple_of(c * CK, CK), CK)])
                a = a + jnp.dot(vt, p.astype(bf16), preferred_element_type=f32)
                return l + jnp.sum(p, axis=0, keepdims=True), a

            l, a = lax.fori_loop(0, NC, sum_body,
                                 (jnp.zeros((1, TQ), f32), jnp.zeros((DH, TQ), f32)))
            op_ref[pl.ds(h8, 8), cols] = _pack(a * (1.0 / l))
            return carry

        lax.fori_loop(0, NQ * H, unit, 0)

    def out_copy(n):
        rows = pl.ds(0, NV) if n == NP else pl.ds(NV + n * MR, MR)
        return pltpu.make_async_copy(o_ref.at[rows, :], o_hbm.at[rows, :], osem.at[n])

    send_after = {7: range(0, 4), 13: range(4, 7), 15: range(7, NP + 1)}

    def token_spans(c):
        return ((0, c * VK, VK), (VK, NV + c * MK, MK))

    for n in range(3, 8):
        w_copy(n).wait()
    wr = jnp.broadcast_to(wr_ref[pl.ds(0, D)].astype(f32).reshape(1, D), (16, D)).astype(bf16)
    wo = wo_ref[...]

    def out_proj(c):
        ot = _unpack(op_ref[:, c * CK:(c + 1) * CK])
        return lax.dot_general(ot, wo, (((0,), (0,)), ((), ())),
                               preferred_element_type=f32)

    def residual_ln(c, attn):
        xb = jnp.concatenate(
            [x_ref[t0:t0 + n, :].astype(f32) for _, t0, n in token_spans(c)], axis=0)
        h = _rb(xb + attn)
        hn = _layernorm_bf16(h).astype(bf16)
        hnf = hn.astype(f32)
        o = h + hnf
        for p0, t0, n in token_spans(c):
            h_ref[t0:t0 + n, :] = h[p0:p0 + n]
            hn_ref[t0:t0 + n, :] = hnf[p0:p0 + n]
            o_ref[t0:t0 + n, :] = o[p0:p0 + n].astype(bf16)
        for n in send_after.get(c, ()):
            out_copy(n).start()
        return hn

    def router(c, hn):
        r = lax.dot_general(wr, hn, (((1,), (1,)), ((), ())), preferred_element_type=f32)
        r = jnp.clip(_rb(r[0:8, :]), -BF16_MAX, BF16_MAX)
        r = jnp.where(jnp.abs(r) < F32_TINY, F32_TINY, r)
        off = lax.broadcasted_iota(i32, r.shape, 1)
        tok = off + jnp.where(off < VK, c * VK, NV + c * MK - VK)
        key = pltpu.bitcast(r, i32) | jnp.where(r < 0, tok, S - 1 - tok)
        return pltpu.bitcast(key, f32)

    attn = out_proj(0)
    hn_prev = None
    keys = []
    for c in range(NC):
        attn_next = out_proj(c + 1) if c + 1 < NC else None
        if hn_prev is not None:
            keys.append(router(c - 1, hn_prev))
        hn_prev = residual_ln(c, attn)
        attn = attn_next
    keys.append(router(NC - 1, hn_prev))

    top, sec = keys[0], jnp.full(keys[0].shape, -jnp.inf, f32)
    for k in keys[1:]:
        sec = jnp.maximum(sec, jnp.minimum(top, k))
        top = jnp.maximum(top, k)
    k1 = jnp.max(top, axis=1, keepdims=True)
    k2 = jnp.max(jnp.where(top == k1, sec, top), axis=1, keepdims=True)

    def decode(k):
        bits = pltpu.bitcast(jnp.broadcast_to(k, (8, 128)), i32)
        low = bits & 0xFFFF
        tok = jnp.where(bits < 0, low, S - 1 - low)
        score = pltpu.bitcast(bits & jnp.int32(-65536), f32)
        return jnp.clip(tok[0, 0], 0, S - 1), score[0:1, 0:1]

    i1, r1 = decode(k1)
    i2, r2 = decode(k2)
    row16 = lax.broadcasted_iota(i32, (16, D), 0)
    first = row16 == 0
    hsel = jnp.where(first, h_ref[pl.ds(i1, 1), :], h_ref[pl.ds(i2, 1), :])
    xsel = jnp.where(first, hn_ref[pl.ds(i1, 1), :], hn_ref[pl.ds(i2, 1), :])
    xs = xsel.astype(bf16)
    gpre = _rb(jnp.dot(xs, wg_ref[...], preferred_element_type=f32))
    gate = _rb(gpre * jax.nn.sigmoid(gpre))
    up = _rb(jnp.dot(xs, wu_ref[...], preferred_element_type=f32))
    y = _rb(jnp.dot((gate * up).astype(bf16), wd_ref[...], preferred_element_type=f32))
    y = _rb(y * _rb(jax.nn.sigmoid(jnp.where(first, r1, r2))))
    osel = hsel + _rb(xsel + y)
    for n in range(NP + 1):
        out_copy(n).wait()
    bases = [pl.multiple_of(lax.shift_right_logical(idx, 4) * 16, 16) for idx in (i1, i2)]
    olds = [o_ref[pl.ds(base, 16), :].astype(f32) for base in bases]
    for base, old in zip(bases, olds):
        t = row16 + base
        new = jnp.where(t == i1, osel[0:1, :], jnp.where(t == i2, osel[1:2, :], old))
        o_ref[pl.ds(base, 16), :] = new.astype(bf16)
    patch = [pltpu.make_async_copy(o_ref.at[pl.ds(base, 16), :], o_hbm.at[pl.ds(base, 16), :],
                                   osem.at[n]) for n, base in enumerate(bases)]
    patch[0].start()

    @pl.when(bases[0] != bases[1])
    def _():
        patch[1].start()
        patch[1].wait()

    patch[0].wait()


@jax.jit
def pallas_sequential_preLN__mha_block__moe_arch_mod__prompt_kernel(
    A_x: jax.Array,
    A_wqkv: jax.Array,
    A_wo: jax.Array,
    B_x: jax.Array,
    B_w_r: jax.Array,
    B_w_gate: jax.Array,
    B_w_up: jax.Array,
    B_w_down: jax.Array,
):
    B, S, D = A_x.shape
    F = B_w_gate.shape[1]
    assert B == 1 and D == H * DH and S == 2048
    hbm = pl.BlockSpec(memory_space=pl.ANY)
    NC = S // CK
    NV = NC * VK
    out = pl.pallas_call(
        _kernel,
        out_shape=jax.ShapeDtypeStruct((S, D), A_x.dtype),
        in_specs=[hbm] * 7,
        out_specs=hbm,
        scratch_shapes=[
            pltpu.VMEM((S, D), bf16),
            pltpu.VMEM((S // 2, D), u32),
            pltpu.VMEM((D, 3 * D), bf16),
            pltpu.VMEM((2 * D, D), bf16),
            pltpu.VMEM((H // HG, NC * MK // 2, 128), u32),
            pltpu.VMEM((H // HG, NV // 2, 128), u32),
            pltpu.VMEM((128, H // HG, NV, 128), f32),
            pltpu.VMEM((D // 2, S), u32),
            pltpu.VMEM((D // 2, S), u32),
            pltpu.VMEM((D // 2, S), u32),
            pltpu.VMEM((H, S), f32),
            pltpu.VMEM((S, D), f32),
            pltpu.VMEM((S, D), f32),
            pltpu.VMEM((S, D), bf16),
            pltpu.VMEM((D, D), bf16),
            pltpu.VMEM((D, F), bf16),
            pltpu.VMEM((D, F), bf16),
            pltpu.VMEM((F, D), bf16),
            pltpu.VMEM((16 * D,), bf16),
            pltpu.SemaphoreType.DMA((3,)),
            pltpu.SemaphoreType.DMA((8,)),
            pltpu.SemaphoreType.DMA((S // TP + 1,)),
        ] + [pltpu.VMEM((CK // 2, TQ), u32)] * RING + [pltpu.VMEM((DH, 8, TQ), f32)] * HG,
        compiler_params=pltpu.CompilerParams(vmem_limit_bytes=120 * 1024 * 1024),
    )(A_x.reshape(S, D), A_wqkv, B_w_r, A_wo, B_w_gate, B_w_up, B_w_down)
    return out.reshape(B, S, D)
```

```python
import math

import jax
import jax.numpy as jnp
from jax import lax
import jax.experimental.pallas as pl
import jax.experimental.pallas.tpu as pltpu

f32, bf16, u32, i32 = jnp.float32, jnp.bfloat16, jnp.uint32, jnp.int32

H = 32
DH = 16
HG = 8
TQ = 512
CK = 128
VK = 16
MK = CK - VK
LAG = 4
RING = 8
TP = 2 * CK
EPS = 1e-5
BF16_MAX = 3.3895313892515355e38
F32_TINY = 2.0 ** -126
L_LO, L_HI = 2.0 ** -60, 2.0 ** 60


def _rb(x):
    return x.astype(bf16).astype(f32)


def _mean(x):
    return jnp.sum(x, axis=-1, keepdims=True) * (1.0 / x.shape[-1])


def _layernorm(x):
    xc = x - _mean(x)
    return xc * lax.rsqrt(_mean(xc * xc) + EPS)


def _layernorm_bf16(x):
    mean = _mean(x)
    xc = x - mean
    v = _rb(_rb(_mean(xc * xc)) + EPS)
    den = _rb(v * lax.rsqrt(v))
    inv = pl.reciprocal(den, approx=True)
    inv = inv * (2.0 - den * inv)
    return (x - _rb(mean)) * inv


def _pack(x):
    return pltpu.bitcast(x.astype(bf16), u32)


def _unpack(x):
    return pltpu.bitcast(x, bf16)


def _kernel(x_hbm, wqkv_hbm, wr_hbm, wo_hbm, wg_hbm, wu_hbm, wd_hbm, o_hbm,
            x_ref, xn_ref, wqkv_ref, wt_ref, kp_ref, kv_ref, kb_ref, qp_ref, vp_ref, op_ref,
            l_ref, h_ref, hn_ref, o_ref, wo_ref, wg_ref, wu_ref, wd_ref, wr_ref,
            xsem, wsem, osem, *stage):
    pt_refs = stage[:RING]
    qs_refs = stage[RING:]
    S, D = x_ref.shape
    NQ = S // TQ
    NC = S // CK
    NG = H // HG
    NP = S // TP
    NV = NC * VK
    MR = 2 * MK

    B0, B1 = 1, 5
    x_cuts = (0, NV + B0 * MR, NV + B1 * MR, S)

    def x_copy(n):
        rows = pl.ds(x_cuts[n], x_cuts[n + 1] - x_cuts[n])
        return pltpu.make_async_copy(x_hbm.at[rows, :], x_ref.at[rows, :], xsem.at[n])

    def w_copy(n):
        if n < 3:
            cols = pl.ds(n * D, D)
            return pltpu.make_async_copy(wqkv_hbm.at[:, cols], wqkv_ref.at[:, cols], wsem.at[n])
        src, dst = ((wo_hbm, wo_ref), (wg_hbm, wg_ref), (wu_hbm, wu_ref), (wd_hbm, wd_ref),
                    (wr_hbm, wr_ref.at[pl.ds(0, D)]))[n - 3]
        return pltpu.make_async_copy(src, dst, wsem.at[n])

    x_copy(0).start()
    w_copy(1).start()
    x_copy(1).start()
    x_copy(2).start()
    w_copy(0).start()
    w_copy(2).start()

    def bcast_keys(jds):
        for jd in jds:
            col = jnp.broadcast_to(kv_ref[:, :, jd:jd + 1], kv_ref.shape)
            kb_ref[jd] = _unpack(col).astype(f32)

    def ln_block(b):
        xn = _layernorm(x_ref[NV + b * MR:NV + (b + 1) * MR, :].astype(f32))
        xu = _pack(xn)
        for cc in range(2):
            r0 = (2 * b + cc) * (CK // 2) + VK // 2
            xn_ref[r0:r0 + MK // 2, :] = xu[cc * (MK // 2):(cc + 1) * (MK // 2)]

    def k_proj(b):
        xu = jnp.concatenate(
            [xn_ref[(2 * b + cc) * (CK // 2) + VK // 2:(2 * b + cc + 1) * (CK // 2), :]
             for cc in range(2)], axis=0)
        k = jnp.dot(_unpack(xu), wqkv_ref[:, D:2 * D], preferred_element_type=f32)
        for g in range(NG):
            kp_ref[g, b * MK:(b + 1) * MK, :] = _pack(k[:, g * 128:(g + 1) * 128])

    early = 4
    jds = [j * DH + d for d in range(early) for j in range(HG)]

    x_copy(0).wait()
    xu0 = _pack(_layernorm(x_ref[0:NV, :].astype(f32)))
    for c in range(NC):
        xn_ref[c * (CK // 2):c * (CK // 2) + VK // 2, :] = xu0[c * 8:(c + 1) * 8]
    for b in range(B0):
        ln_block(b)
    w_copy(1).wait()
    kv = jnp.dot(_unpack(xu0), wqkv_ref[:, D:2 * D], preferred_element_type=f32)
    for g in range(NG):
        kv_ref[g] = _pack(kv[:, g * 128:(g + 1) * 128])
    bcast_keys(jds[:8])
    x_copy(1).wait()
    for b in range(B0, B1):
        ln_block(b)
    bcast_keys(jds[8:23])
    for b in range(B1 - 1):
        k_proj(b)
    x_copy(2).wait()
    w_copy(0).wait()
    w_copy(2).wait()
    for n in range(3, 8):
        w_copy(n).start()
    for b in range(B1, NP):
        ln_block(b)
    wt_ref[0:D // 2, :] = _pack(wqkv_ref[:, 0:D].astype(f32).T)
    wt_ref[D // 2:D, :] = _pack(wqkv_ref[:, 2 * D:3 * D].astype(f32).T)
    bcast_keys(jds[23:])
    for b in range(B1 - 1, NP):
        k_proj(b)
    qscale = (DH ** -0.5) * math.log2(math.e)
    for b in range(NP):
        bcast_keys([b * DH + d for d in range(early, DH)])
        xp = _unpack(xn_ref[b * (TP // 2):(b + 1) * (TP // 2), :])
        qv = lax.dot_general(_unpack(wt_ref[...]), xp, (((1,), (1,)), ((), ())),
                             preferred_element_type=f32)
        qp_ref[:, b * TP:(b + 1) * TP] = _pack(qv[0:D] * qscale)
        vp_ref[:, b * TP:(b + 1) * TP] = _pack(qv[D:2 * D])

    NI = NQ * NG

    def unit_index(i, j):
        h = (i % NG) * HG + j
        return h, pl.multiple_of(h * 8, 8), pl.ds(pl.multiple_of((i // NG) * TQ, TQ), TQ)

    def stage_q(unit, j, lo, hi):
        _, h8, cols = unit
        qf = _unpack(qp_ref[pl.ds(h8, 8), cols]).astype(f32)
        for d in range(lo, hi):
            qs_refs[j][d] = jnp.broadcast_to(qf[d:d + 1, :], (8, TQ))

    def pv_step(unit, c, row0, acc, inv_l, link=None):
        _, h8, cols = unit
        vt = _unpack(vp_ref[pl.ds(h8, 8), c * CK:(c + 1) * CK])
        d = jnp.dot(vt, _unpack(pt_refs[c % RING][pl.ds(row0, CK // 2), :]),
                    preferred_element_type=f32)
        if acc is None:
            acc = jnp.where(link[0], link[1], d)
        else:
            acc = acc + d
        if c == NC - 1:
            op_ref[pl.ds(h8, 8), cols] = _pack(acc * jnp.concatenate([inv_l, inv_l], axis=0))
        return acc

    def inv_denominator(unit, l8):
        h, _, cols = unit
        l = jnp.sum(l8, axis=0, keepdims=True)
        l_ref[pl.ds(h, 1), cols] = l
        inv = pl.reciprocal(l, approx=True)
        inv = inv * (2.0 - l * inv)
        return jnp.broadcast_to(inv, l8.shape)

    def fast_group(i, carry):
        z1 = lax.shift_right_logical(i, 20)
        row0 = pl.multiple_of(z1 * 8, 8)
        never = lax.broadcasted_iota(i32, (VK, 128), 0) < z1
        never_wide = lax.broadcasted_iota(i32, (DH, TQ), 0) < z1
        g = i % NG
        units = {j: unit_index(i, j) for j in range(HG)}
        units[-1] = unit_index((i + NI - 1) % NI, HG - 1)
        units[HG] = unit_index(jnp.minimum(i + 1, NI - 1), 0)
        dims = [z1 + d0 for d0 in range(0, DH, 4)]
        acc = {-1: carry[0]}
        l8 = {-1: inv_denominator(units[-1], carry[1])}
        pend = [(-1, c) for c in range(NC - LAG, NC)]
        prev = None
        for j in range(HG):
            _, h8, cols = units[j]
            kdims = [d0 + j * DH for d0 in dims]
            qrow = qp_ref[pl.ds(h8, 8), cols]
            z = jnp.zeros_like(qrow)
            w = _unpack(jnp.concatenate([qrow if b == j else z for b in range(HG)], axis=0))
            acc[j] = None
            l8[j] = None
            jn = (j + 1) % HG
            for c in range(NC):
                pt_ref = pt_refs[c % RING]
                base = c * (MK // 2)
                kc = _unpack(jnp.concatenate(
                    [kp_ref[g, base + b * 8:base + (b + 1) * 8, :] for b in range(6, -1, -1)],
                    axis=0))
                p = jnp.exp2(jnp.dot(kc, w, preferred_element_type=f32))
                cl = jnp.sum(p.reshape(MK // 8, 8, TQ), axis=0)
                l8[j] = cl if l8[j] is None else l8[j] + cl
                for b in range(7):
                    pt_ref[(7 - b) * 8:(8 - b) * 8, :] = _pack(p[b * 16:(b + 1) * 16, :])
                pend.append((j, c))
                pj, pc = pend.pop(0)
                link = (never_wide, acc[pj - 1]) if pc == 0 else None
                acc[pj] = pv_step(units[pj], pc, row0, acc[pj], l8[pj], link)

                tie = None
                if c in (7, 9, 11, 13):
                    tie = qs_refs[jn][z1, :, 0:128]
                    tie = jnp.concatenate([tie, tie], axis=0)
                tiles = []
                for t in range(TQ // 128):
                    a = None
                    for d0, kd0 in zip(dims, kdims):
                        kb = kb_ref[pl.ds(kd0, 4), g, c * VK:(c + 1) * VK, :]
                        qd = qs_refs[j][pl.ds(d0, 4), :, t * 128:(t + 1) * 128]
                        pr = kb * jnp.concatenate([qd, qd], axis=1)
                        if a is not None:
                            a = jnp.sum(jnp.concatenate([a[None], pr], axis=0), axis=0)
                            continue
                        a = pr[0]
                        if t == 0 and tie is not None:
                            a = jnp.where(never, tie, a)
                        a = a + pr[1] + pr[2]
                        if prev is not None:
                            a = jnp.where(never, prev, a)
                        a = a + pr[3]
                    prev = a
                    tiles.append(a)
                p = jnp.exp2(jnp.concatenate(tiles, axis=1))
                l8[j] = l8[j] + (p[0:8] + p[8:16])
                pt_ref[0:8, :] = _pack(p)
                if c == NC - 1 and j < HG - 1:
                    l8[j] = inv_denominator(units[j], l8[j])
                if c in (6, 8, 10, 12):
                    stage_q(units[j + 1], jn, (c - 6) * 2, (c - 6) * 2 + 4)
        return acc[HG - 1], l8[HG - 1]

    stage_q(unit_index(0, 0), 0, 0, DH)
    for c in range(NC - LAG, NC):
        pt_refs[c % RING][...] = jnp.zeros((CK // 2, TQ), u32)
    acc, l8 = lax.fori_loop(0, NI, fast_group,
                            (jnp.zeros((DH, TQ), f32), jnp.ones((8, TQ), f32)))
    inv_l = inv_denominator(unit_index(NI - 1, HG - 1), l8)
    for c in range(NC - LAG, NC):
        acc = pv_step(unit_index(NI - 1, HG - 1), c, 0, acc, inv_l)

    l_all = l_ref[...]
    safe = jnp.logical_and(jnp.min(l_all) >= L_LO, jnp.max(l_all) <= L_HI)

    @pl.when(jnp.logical_not(safe))
    def _():
        def unit(u, carry):
            h = u % H
            g = h // HG
            j = h % HG
            cols = pl.ds(pl.multiple_of((u // H) * TQ, TQ), TQ)
            h8 = pl.multiple_of(h * 8, 8)
            qrow = qp_ref[pl.ds(h8, 8), cols]
            z = jnp.zeros_like(qrow)
            w = _unpack(jnp.concatenate(
                [jnp.where(j == b, qrow, z) for b in range(HG)], axis=0))

            def scores(c):
                kc = jnp.concatenate(
                    [kv_ref[g, pl.ds(pl.multiple_of(c * 8, 8), 8), :],
                     kp_ref[g, pl.ds(pl.multiple_of(c * (MK // 2), 8), MK // 2), :]], axis=0)
                return jnp.dot(_unpack(kc), w, preferred_element_type=f32)

            def max_body(c, m):
                return jnp.maximum(m, jnp.max(scores(c), axis=0, keepdims=True))

            m = lax.fori_loop(0, NC, max_body, jnp.full((1, TQ), -jnp.inf, f32))

            def sum_body(c, la):
                l, a = la
                p = jnp.exp2(scores(c) - m)
                vt = _unpack(vp_ref[pl.ds(h8, 8), pl.ds(pl.multiple_of(c * CK, CK), CK)])
                a = a + jnp.dot(vt, p.astype(bf16), preferred_element_type=f32)
                return l + jnp.sum(p, axis=0, keepdims=True), a

            l, a = lax.fori_loop(0, NC, sum_body,
                                 (jnp.zeros((1, TQ), f32), jnp.zeros((DH, TQ), f32)))
            op_ref[pl.ds(h8, 8), cols] = _pack(a * (1.0 / l))
            return carry

        lax.fori_loop(0, NQ * H, unit, 0)

    def out_copy(n):
        rows = pl.ds(0, NV) if n == NP else pl.ds(NV + n * MR, MR)
        return pltpu.make_async_copy(o_ref.at[rows, :], o_hbm.at[rows, :], osem.at[n])

    send_after = {7: range(0, 4), 13: range(4, 7), 15: range(7, NP + 1)}

    def token_spans(c):
        return ((0, c * VK, VK), (VK, NV + c * MK, MK))

    for n in range(3, 8):
        w_copy(n).wait()
    wr = jnp.broadcast_to(wr_ref[pl.ds(0, D)].astype(f32).reshape(1, D), (16, D)).astype(bf16)
    wo = wo_ref[...]

    def out_proj(c):
        ot = _unpack(op_ref[:, c * CK:(c + 1) * CK])
        return lax.dot_general(ot, wo, (((0,), (0,)), ((), ())),
                               preferred_element_type=f32)

    def residual_ln(c, attn):
        xb = jnp.concatenate(
            [x_ref[t0:t0 + n, :].astype(f32) for _, t0, n in token_spans(c)], axis=0)
        h = _rb(xb + attn)
        hn = _layernorm_bf16(h).astype(bf16)
        hnf = hn.astype(f32)
        o = h + hnf
        for p0, t0, n in token_spans(c):
            h_ref[t0:t0 + n, :] = h[p0:p0 + n]
            hn_ref[t0:t0 + n, :] = hnf[p0:p0 + n]
            o_ref[t0:t0 + n, :] = o[p0:p0 + n].astype(bf16)
        for n in send_after.get(c, ()):
            out_copy(n).start()
        return hn

    def router(c, hn):
        r = lax.dot_general(wr, hn, (((1,), (1,)), ((), ())), preferred_element_type=f32)
        r = jnp.clip(_rb(r[0:8, :]), -BF16_MAX, BF16_MAX)
        r = jnp.where(jnp.abs(r) < F32_TINY, F32_TINY, r)
        off = lax.broadcasted_iota(i32, r.shape, 1)
        tok = off + jnp.where(off < VK, c * VK, NV + c * MK - VK)
        key = pltpu.bitcast(r, i32) | jnp.where(r < 0, tok, S - 1 - tok)
        return pltpu.bitcast(key, f32)

    attn = out_proj(0)
    hn_prev = None
    keys = []
    for c in range(NC):
        attn_next = out_proj(c + 1) if c + 1 < NC else None
        if hn_prev is not None:
            keys.append(router(c - 1, hn_prev))
        hn_prev = residual_ln(c, attn)
        attn = attn_next
    keys.append(router(NC - 1, hn_prev))

    top, sec = keys[0], jnp.full(keys[0].shape, -jnp.inf, f32)
    for k in keys[1:]:
        sec = jnp.maximum(sec, jnp.minimum(top, k))
        top = jnp.maximum(top, k)
    k1 = jnp.max(top, axis=1, keepdims=True)
    k2 = jnp.max(jnp.where(top == k1, sec, top), axis=1, keepdims=True)

    def decode(k):
        bits = pltpu.bitcast(jnp.broadcast_to(k, (8, 128)), i32)
        low = bits & 0xFFFF
        tok = jnp.where(bits < 0, low, S - 1 - low)
        score = pltpu.bitcast(bits & jnp.int32(-65536), f32)
        return jnp.clip(tok[0, 0], 0, S - 1), score[0:1, 0:1]

    i1, r1 = decode(k1)
    i2, r2 = decode(k2)
    row16 = lax.broadcasted_iota(i32, (16, D), 0)
    first = row16 == 0
    hsel = jnp.where(first, h_ref[pl.ds(i1, 1), :], h_ref[pl.ds(i2, 1), :])
    xsel = jnp.where(first, hn_ref[pl.ds(i1, 1), :], hn_ref[pl.ds(i2, 1), :])
    xs = xsel.astype(bf16)
    gpre = _rb(jnp.dot(xs, wg_ref[...], preferred_element_type=f32))
    gate = _rb(gpre * jax.nn.sigmoid(gpre))
    up = _rb(jnp.dot(xs, wu_ref[...], preferred_element_type=f32))
    y = _rb(jnp.dot((gate * up).astype(bf16), wd_ref[...], preferred_element_type=f32))
    y = _rb(y * _rb(jax.nn.sigmoid(jnp.where(first, r1, r2))))
    osel = hsel + _rb(xsel + y)
    for n in range(NP + 1):
        out_copy(n).wait()
    bases = [pl.multiple_of(lax.shift_right_logical(idx, 4) * 16, 16) for idx in (i1, i2)]
    olds = [o_ref[pl.ds(base, 16), :].astype(f32) for base in bases]
    for base, old in zip(bases, olds):
        t = row16 + base
        new = jnp.where(t == i1, osel[0:1, :], jnp.where(t == i2, osel[1:2, :], old))
        o_ref[pl.ds(base, 16), :] = new.astype(bf16)
    patch = [pltpu.make_async_copy(o_ref.at[pl.ds(base, 16), :], o_hbm.at[pl.ds(base, 16), :],
                                   osem.at[n]) for n, base in enumerate(bases)]
    patch[0].start()

    @pl.when(bases[0] != bases[1])
    def _():
        patch[1].start()
        patch[1].wait()

    patch[0].wait()


@jax.jit
def pallas_sequential_preLN__mha_block__moe_arch_mod__prompt_kernel(
    A_x: jax.Array,
    A_wqkv: jax.Array,
    A_wo: jax.Array,
    B_x: jax.Array,
    B_w_r: jax.Array,
    B_w_gate: jax.Array,
    B_w_up: jax.Array,
    B_w_down: jax.Array,
):
    B, S, D = A_x.shape
    F = B_w_gate.shape[1]
    assert B == 1 and D == H * DH and S == 2048
    hbm = pl.BlockSpec(memory_space=pl.ANY)
    NC = S // CK
    NV = NC * VK
    out = pl.pallas_call(
        _kernel,
        out_shape=jax.ShapeDtypeStruct((S, D), A_x.dtype),
        in_specs=[hbm] * 7,
        out_specs=hbm,
        scratch_shapes=[
            pltpu.VMEM((S, D), bf16),
            pltpu.VMEM((S // 2, D), u32),
            pltpu.VMEM((D, 3 * D), bf16),
            pltpu.VMEM((D, D), u32),
            pltpu.VMEM((H // HG, NC * MK // 2, 128), u32),
            pltpu.VMEM((H // HG, NV // 2, 128), u32),
            pltpu.VMEM((128, H // HG, NV, 128), f32),
            pltpu.VMEM((D // 2, S), u32),
            pltpu.VMEM((D // 2, S), u32),
            pltpu.VMEM((D // 2, S), u32),
            pltpu.VMEM((H, S), f32),
            pltpu.VMEM((S, D), f32),
            pltpu.VMEM((S, D), f32),
            pltpu.VMEM((S, D), bf16),
            pltpu.VMEM((D, D), bf16),
            pltpu.VMEM((D, F), bf16),
            pltpu.VMEM((D, F), bf16),
            pltpu.VMEM((F, D), bf16),
            pltpu.VMEM((16 * D,), bf16),
            pltpu.SemaphoreType.DMA((3,)),
            pltpu.SemaphoreType.DMA((8,)),
            pltpu.SemaphoreType.DMA((S // TP + 1,)),
        ] + [pltpu.VMEM((CK // 2, TQ), u32)] * RING + [pltpu.VMEM((DH, 8, TQ), f32)] * HG,
        compiler_params=pltpu.CompilerParams(vmem_limit_bytes=120 * 1024 * 1024),
    )(A_x.reshape(S, D), A_wqkv, B_w_r, A_wo, B_w_gate, B_w_up, B_w_down)
    return out.reshape(B, S, D)
```

```python
import math

import jax
import jax.numpy as jnp
from jax import lax
import jax.experimental.pallas as pl
import jax.experimental.pallas.tpu as pltpu

f32, bf16, u32, i32 = jnp.float32, jnp.bfloat16, jnp.uint32, jnp.int32

H = 32
DH = 16
HG = 8
TQ = 512
CK = 128
VK = 16
MK = CK - VK
LAG = 4
RING = 8
TP = 2 * CK
EPS = 1e-5
BF16_MAX = 3.3895313892515355e38
F32_TINY = 2.0 ** -126
L_LO, L_HI = 2.0 ** -60, 2.0 ** 60


def _rb(x):
    return x.astype(bf16).astype(f32)


def _mean(x):
    return jnp.sum(x, axis=-1, keepdims=True) * (1.0 / x.shape[-1])


def _layernorm(x):
    xc = x - _mean(x)
    return xc * lax.rsqrt(_mean(xc * xc) + EPS)


def _layernorm_bf16(x):
    mean = _mean(x)
    xc = x - mean
    v = _rb(_rb(_mean(xc * xc)) + EPS)
    den = _rb(v * lax.rsqrt(v))
    inv = pl.reciprocal(den, approx=True)
    inv = inv * (2.0 - den * inv)
    return (x - _rb(mean)) * inv


def _pack(x):
    return pltpu.bitcast(x.astype(bf16), u32)


def _unpack(x):
    return pltpu.bitcast(x, bf16)


def _kernel(x_hbm, wqkv_hbm, wr_hbm, wo_hbm, wg_hbm, wu_hbm, wd_hbm, o_hbm,
            x_ref, xn_ref, wqkv_ref, wt_ref, kp_ref, kv_ref, kb_ref, qp_ref, vp_ref, op_ref,
            l_ref, h_ref, hn_ref, o_ref, wo_ref, wg_ref, wu_ref, wd_ref, wr_ref,
            xsem, wsem, osem, *stage):
    pt_refs = stage[:RING]
    qs_refs = stage[RING:]
    S, D = x_ref.shape
    NQ = S // TQ
    NC = S // CK
    NG = H // HG
    NP = S // TP
    NV = NC * VK
    MR = 2 * MK

    B0, B1 = 1, 5
    x_cuts = (0, NV + B0 * MR, NV + B1 * MR, S)

    def x_copy(n):
        rows = pl.ds(x_cuts[n], x_cuts[n + 1] - x_cuts[n])
        return pltpu.make_async_copy(x_hbm.at[rows, :], x_ref.at[rows, :], xsem.at[n])

    def w_copy(n):
        if n < 3:
            cols = pl.ds(n * D, D)
            return pltpu.make_async_copy(wqkv_hbm.at[:, cols], wqkv_ref.at[:, cols], wsem.at[n])
        src, dst = ((wo_hbm, wo_ref), (wg_hbm, wg_ref), (wu_hbm, wu_ref), (wd_hbm, wd_ref),
                    (wr_hbm, wr_ref.at[pl.ds(0, D)]))[n - 3]
        return pltpu.make_async_copy(src, dst, wsem.at[n])

    x_copy(0).start()
    w_copy(1).start()
    x_copy(1).start()
    x_copy(2).start()
    w_copy(0).start()
    w_copy(2).start()

    def bcast_keys(jds):
        for jd in jds:
            col = jnp.broadcast_to(kv_ref[:, :, jd:jd + 1], kv_ref.shape)
            kb_ref[jd] = _unpack(col).astype(f32)

    def ln_block(b):
        xn = _layernorm(x_ref[NV + b * MR:NV + (b + 1) * MR, :].astype(f32))
        for cc in range(2):
            r0 = (2 * b + cc) * (CK // 2) + VK // 2
            xn_ref[r0:r0 + MK // 2, :] = _pack(xn[cc * MK:(cc + 1) * MK])

    def k_proj(b):
        xu = jnp.concatenate(
            [xn_ref[(2 * b + cc) * (CK // 2) + VK // 2:(2 * b + cc + 1) * (CK // 2), :]
             for cc in range(2)], axis=0)
        k = jnp.dot(_unpack(xu), wqkv_ref[:, D:2 * D], preferred_element_type=f32)
        for g in range(NG):
            kp_ref[g, b * MK:(b + 1) * MK, :] = _pack(k[:, g * 128:(g + 1) * 128])

    early = 4
    jds = [j * DH + d for d in range(early) for j in range(HG)]

    x_copy(0).wait()
    xn0 = _layernorm(x_ref[0:NV, :].astype(f32))
    for c in range(NC):
        xn_ref[c * (CK // 2):c * (CK // 2) + VK // 2, :] = _pack(xn0[c * VK:(c + 1) * VK])
    for b in range(B0):
        ln_block(b)
    w_copy(1).wait()
    kv = jnp.dot(xn0.astype(bf16), wqkv_ref[:, D:2 * D], preferred_element_type=f32)
    for g in range(NG):
        kv_ref[g] = _pack(kv[:, g * 128:(g + 1) * 128])
    bcast_keys(jds[:8])
    x_copy(1).wait()
    for b in range(B0, B1):
        ln_block(b)
    bcast_keys(jds[8:23])
    for b in range(B1 - 1):
        k_proj(b)
    x_copy(2).wait()
    w_copy(0).wait()
    w_copy(2).wait()
    for n in range(3, 8):
        w_copy(n).start()
    for b in range(B1, NP):
        ln_block(b)
    wt_ref[0:D // 2, :] = _pack(wqkv_ref[:, 0:D].astype(f32).T)
    wt_ref[D // 2:D, :] = _pack(wqkv_ref[:, 2 * D:3 * D].astype(f32).T)
    bcast_keys(jds[23:])
    for b in range(B1 - 1, NP):
        k_proj(b)
    qscale = (DH ** -0.5) * math.log2(math.e)
    for b in range(NP):
        bcast_keys([b * DH + d for d in range(early, DH)])
        xp = _unpack(xn_ref[b * (TP // 2):(b + 1) * (TP // 2), :])
        qv = lax.dot_general(_unpack(wt_ref[...]), xp, (((1,), (1,)), ((), ())),
                             preferred_element_type=f32)
        qp_ref[:, b * TP:(b + 1) * TP] = _pack(qv[0:D] * qscale)
        vp_ref[:, b * TP:(b + 1) * TP] = _pack(qv[D:2 * D])

    NI = NQ * NG

    def unit_index(i, j):
        h = (i % NG) * HG + j
        return h, pl.multiple_of(h * 8, 8), pl.ds(pl.multiple_of((i // NG) * TQ, TQ), TQ)

    def stage_q(unit, j, lo, hi):
        _, h8, cols = unit
        qf = _unpack(qp_ref[pl.ds(h8, 8), cols]).astype(f32)
        for d in range(lo, hi):
            qs_refs[j][d] = jnp.broadcast_to(qf[d:d + 1, :], (8, TQ))

    def pv_step(unit, c, row0, acc, inv_l, link=None):
        _, h8, cols = unit
        vt = _unpack(vp_ref[pl.ds(h8, 8), c * CK:(c + 1) * CK])
        d = jnp.dot(vt, _unpack(pt_refs[c % RING][pl.ds(row0, CK // 2), :]),
                    preferred_element_type=f32)
        if acc is None:
            acc = jnp.where(link[0], link[1], d)
        else:
            acc = acc + d
        if c == NC - 1:
            op_ref[pl.ds(h8, 8), cols] = _pack(acc * jnp.concatenate([inv_l, inv_l], axis=0))
        return acc

    def inv_denominator(unit, l8):
        h, _, cols = unit
        l = jnp.sum(l8, axis=0, keepdims=True)
        l_ref[pl.ds(h, 1), cols] = l
        inv = pl.reciprocal(l, approx=True)
        inv = inv * (2.0 - l * inv)
        return jnp.broadcast_to(inv, l8.shape)

    def fast_group(i, carry):
        z1 = lax.shift_right_logical(i, 20)
        row0 = pl.multiple_of(z1 * 8, 8)
        never = lax.broadcasted_iota(i32, (VK, 128), 0) < z1
        never_wide = lax.broadcasted_iota(i32, (DH, TQ), 0) < z1
        g = i % NG
        units = {j: unit_index(i, j) for j in range(HG)}
        units[-1] = unit_index((i + NI - 1) % NI, HG - 1)
        units[HG] = unit_index(jnp.minimum(i + 1, NI - 1), 0)
        dims = [z1 + d0 for d0 in range(0, DH, 4)]
        acc = {-1: carry[0]}
        l8 = {-1: inv_denominator(units[-1], carry[1])}
        pend = [(-1, c) for c in range(NC - LAG, NC)]
        prev = None
        for j in range(HG):
            _, h8, cols = units[j]
            kdims = [d0 + j * DH for d0 in dims]
            qrow = qp_ref[pl.ds(h8, 8), cols]
            z = jnp.zeros_like(qrow)
            w = _unpack(jnp.concatenate([qrow if b == j else z for b in range(HG)], axis=0))
            acc[j] = None
            l8[j] = None
            jn = (j + 1) % HG
            for c in range(NC):
                pt_ref = pt_refs[c % RING]
                base = c * (MK // 2)
                kc = _unpack(jnp.concatenate(
                    [kp_ref[g, base + b * 8:base + (b + 1) * 8, :] for b in range(6, -1, -1)],
                    axis=0))
                p = jnp.exp2(jnp.dot(kc, w, preferred_element_type=f32))
                cl = jnp.sum(p.reshape(MK // 8, 8, TQ), axis=0)
                l8[j] = cl if l8[j] is None else l8[j] + cl
                for b in range(7):
                    pt_ref[(7 - b) * 8:(8 - b) * 8, :] = _pack(p[b * 16:(b + 1) * 16, :])
                pend.append((j, c))
                pj, pc = pend.pop(0)
                link = (never_wide, acc[pj - 1]) if pc == 0 else None
                acc[pj] = pv_step(units[pj], pc, row0, acc[pj], l8[pj], link)

                tie = None
                if c in (7, 9, 11, 13):
                    tie = qs_refs[jn][z1, :, 0:128]
                    tie = jnp.concatenate([tie, tie], axis=0)
                tiles = []
                for t in range(TQ // 128):
                    a = None
                    for d0, kd0 in zip(dims, kdims):
                        kb = kb_ref[pl.ds(kd0, 4), g, c * VK:(c + 1) * VK, :]
                        qd = qs_refs[j][pl.ds(d0, 4), :, t * 128:(t + 1) * 128]
                        pr = kb * jnp.concatenate([qd, qd], axis=1)
                        if a is not None:
                            a = jnp.sum(jnp.concatenate([a[None], pr], axis=0), axis=0)
                            continue
                        a = pr[0]
                        if t == 0 and tie is not None:
                            a = jnp.where(never, tie, a)
                        a = a + pr[1] + pr[2]
                        if prev is not None:
                            a = jnp.where(never, prev, a)
                        a = a + pr[3]
                    prev = a
                    tiles.append(a)
                p = jnp.exp2(jnp.concatenate(tiles, axis=1))
                l8[j] = l8[j] + (p[0:8] + p[8:16])
                pt_ref[0:8, :] = _pack(p)
                if c == NC - 1 and j < HG - 1:
                    l8[j] = inv_denominator(units[j], l8[j])
                if c in (6, 8, 10, 12):
                    stage_q(units[j + 1], jn, (c - 6) * 2, (c - 6) * 2 + 4)
        return acc[HG - 1], l8[HG - 1]

    stage_q(unit_index(0, 0), 0, 0, DH)
    for c in range(NC - LAG, NC):
        pt_refs[c % RING][...] = jnp.zeros((CK // 2, TQ), u32)
    acc, l8 = lax.fori_loop(0, NI, fast_group,
                            (jnp.zeros((DH, TQ), f32), jnp.ones((8, TQ), f32)))
    inv_l = inv_denominator(unit_index(NI - 1, HG - 1), l8)
    for c in range(NC - LAG, NC):
        acc = pv_step(unit_index(NI - 1, HG - 1), c, 0, acc, inv_l)

    l_all = l_ref[...]
    in_window = jnp.logical_and(l_all >= L_LO, l_all <= L_HI)

    @pl.when(jnp.max(jnp.where(in_window, 0.0, 1.0)) > 0.0)
    def _():
        def unit(u, carry):
            h = u % H
            g = h // HG
            j = h % HG
            cols = pl.ds(pl.multiple_of((u // H) * TQ, TQ), TQ)
            h8 = pl.multiple_of(h * 8, 8)
            qrow = qp_ref[pl.ds(h8, 8), cols]
            z = jnp.zeros_like(qrow)
            w = _unpack(jnp.concatenate(
                [jnp.where(j == b, qrow, z) for b in range(HG)], axis=0))

            def scores(c):
                kc = jnp.concatenate(
                    [kv_ref[g, pl.ds(pl.multiple_of(c * 8, 8), 8), :],
                     kp_ref[g, pl.ds(pl.multiple_of(c * (MK // 2), 8), MK // 2), :]], axis=0)
                return jnp.dot(_unpack(kc), w, preferred_element_type=f32)

            def max_body(c, m):
                return jnp.maximum(m, jnp.max(scores(c), axis=0, keepdims=True))

            m = lax.fori_loop(0, NC, max_body, jnp.full((1, TQ), -jnp.inf, f32))

            def sum_body(c, la):
                l, a = la
                p = jnp.exp2(scores(c) - m)
                vt = _unpack(vp_ref[pl.ds(h8, 8), pl.ds(pl.multiple_of(c * CK, CK), CK)])
                a = a + jnp.dot(vt, p.astype(bf16), preferred_element_type=f32)
                return l + jnp.sum(p, axis=0, keepdims=True), a

            l, a = lax.fori_loop(0, NC, sum_body,
                                 (jnp.zeros((1, TQ), f32), jnp.zeros((DH, TQ), f32)))
            op_ref[pl.ds(h8, 8), cols] = _pack(a * (1.0 / l))
            return carry

        lax.fori_loop(0, NQ * H, unit, 0)

    def out_copy(n):
        rows = pl.ds(0, NV) if n == NP else pl.ds(NV + n * MR, MR)
        return pltpu.make_async_copy(o_ref.at[rows, :], o_hbm.at[rows, :], osem.at[n])

    send_after = {7: range(0, 4), 13: range(4, 7), 15: range(7, NP + 1)}

    def token_spans(c):
        return ((0, c * VK, VK), (VK, NV + c * MK, MK))

    for n in range(3, 8):
        w_copy(n).wait()
    wr = jnp.broadcast_to(wr_ref[pl.ds(0, D)].astype(f32).reshape(1, D), (16, D)).astype(bf16)
    wo = wo_ref[...]

    def out_proj(c):
        ot = _unpack(op_ref[:, c * CK:(c + 1) * CK])
        return lax.dot_general(ot, wo, (((0,), (0,)), ((), ())),
                               preferred_element_type=f32)

    def residual_ln(c, attn):
        xb = jnp.concatenate(
            [x_ref[t0:t0 + n, :].astype(f32) for _, t0, n in token_spans(c)], axis=0)
        h = _rb(xb + attn)
        hn = _layernorm_bf16(h).astype(bf16)
        hnf = hn.astype(f32)
        o = h + hnf
        for p0, t0, n in token_spans(c):
            h_ref[t0:t0 + n, :] = h[p0:p0 + n]
            hn_ref[t0:t0 + n, :] = hnf[p0:p0 + n]
            o_ref[t0:t0 + n, :] = o[p0:p0 + n].astype(bf16)
        for n in send_after.get(c, ()):
            out_copy(n).start()
        return hn

    def router(c, hn):
        r = lax.dot_general(wr, hn, (((1,), (1,)), ((), ())), preferred_element_type=f32)
        r = jnp.clip(_rb(r[0:8, :]), -BF16_MAX, BF16_MAX)
        r = jnp.where(jnp.abs(r) < F32_TINY, F32_TINY, r)
        off = lax.broadcasted_iota(i32, r.shape, 1)
        tok = off + jnp.where(off < VK, c * VK, NV + c * MK - VK)
        key = pltpu.bitcast(r, i32) | jnp.where(r < 0, tok, S - 1 - tok)
        return pltpu.bitcast(key, f32)

    attn = out_proj(0)
    hn_prev = None
    keys = []
    for c in range(NC):
        attn_next = out_proj(c + 1) if c + 1 < NC else None
        if hn_prev is not None:
            keys.append(router(c - 1, hn_prev))
        hn_prev = residual_ln(c, attn)
        attn = attn_next
    keys.append(router(NC - 1, hn_prev))

    top, sec = keys[0], jnp.full(keys[0].shape, -jnp.inf, f32)
    for k in keys[1:]:
        sec = jnp.maximum(sec, jnp.minimum(top, k))
        top = jnp.maximum(top, k)
    k1 = jnp.max(top, axis=1, keepdims=True)
    k2 = jnp.max(jnp.where(top == k1, sec, top), axis=1, keepdims=True)

    def decode(k):
        bits = pltpu.bitcast(jnp.broadcast_to(k, (8, 128)), i32)
        low = bits & 0xFFFF
        tok = jnp.where(bits < 0, low, S - 1 - low)
        score = pltpu.bitcast(bits & jnp.int32(-65536), f32)
        return jnp.clip(tok[0, 0], 0, S - 1), score[0:1, 0:1]

    i1, r1 = decode(k1)
    i2, r2 = decode(k2)
    row16 = lax.broadcasted_iota(i32, (16, D), 0)
    first = row16 == 0
    hsel = jnp.where(first, h_ref[pl.ds(i1, 1), :], h_ref[pl.ds(i2, 1), :])
    xsel = jnp.where(first, hn_ref[pl.ds(i1, 1), :], hn_ref[pl.ds(i2, 1), :])
    xs = xsel.astype(bf16)
    gpre = _rb(jnp.dot(xs, wg_ref[...], preferred_element_type=f32))
    gate = _rb(gpre * jax.nn.sigmoid(gpre))
    up = _rb(jnp.dot(xs, wu_ref[...], preferred_element_type=f32))
    y = _rb(jnp.dot((gate * up).astype(bf16), wd_ref[...], preferred_element_type=f32))
    y = _rb(y * _rb(jax.nn.sigmoid(jnp.where(first, r1, r2))))
    osel = hsel + _rb(xsel + y)
    for n in range(NP + 1):
        out_copy(n).wait()
    bases = [pl.multiple_of(lax.shift_right_logical(idx, 4) * 16, 16) for idx in (i1, i2)]
    olds = [o_ref[pl.ds(base, 16), :].astype(f32) for base in bases]
    for base, old in zip(bases, olds):
        t = row16 + base
        new = jnp.where(t == i1, osel[0:1, :], jnp.where(t == i2, osel[1:2, :], old))
        o_ref[pl.ds(base, 16), :] = new.astype(bf16)
    patch = [pltpu.make_async_copy(o_ref.at[pl.ds(base, 16), :], o_hbm.at[pl.ds(base, 16), :],
                                   osem.at[n]) for n, base in enumerate(bases)]
    patch[0].start()

    @pl.when(bases[0] != bases[1])
    def _():
        patch[1].start()
        patch[1].wait()

    patch[0].wait()


@jax.jit
def pallas_sequential_preLN__mha_block__moe_arch_mod__prompt_kernel(
    A_x: jax.Array,
    A_wqkv: jax.Array,
    A_wo: jax.Array,
    B_x: jax.Array,
    B_w_r: jax.Array,
    B_w_gate: jax.Array,
    B_w_up: jax.Array,
    B_w_down: jax.Array,
):
    B, S, D = A_x.shape
    F = B_w_gate.shape[1]
    assert B == 1 and D == H * DH and S == 2048
    hbm = pl.BlockSpec(memory_space=pl.ANY)
    NC = S // CK
    NV = NC * VK
    out = pl.pallas_call(
        _kernel,
        out_shape=jax.ShapeDtypeStruct((S, D), A_x.dtype),
        in_specs=[hbm] * 7,
        out_specs=hbm,
        scratch_shapes=[
            pltpu.VMEM((S, D), bf16),
            pltpu.VMEM((S // 2, D), u32),
            pltpu.VMEM((D, 3 * D), bf16),
            pltpu.VMEM((D, D), u32),
            pltpu.VMEM((H // HG, NC * MK // 2, 128), u32),
            pltpu.VMEM((H // HG, NV // 2, 128), u32),
            pltpu.VMEM((128, H // HG, NV, 128), f32),
            pltpu.VMEM((D // 2, S), u32),
            pltpu.VMEM((D // 2, S), u32),
            pltpu.VMEM((D // 2, S), u32),
            pltpu.VMEM((H, S), f32),
            pltpu.VMEM((S, D), f32),
            pltpu.VMEM((S, D), f32),
            pltpu.VMEM((S, D), bf16),
            pltpu.VMEM((D, D), bf16),
            pltpu.VMEM((D, F), bf16),
            pltpu.VMEM((D, F), bf16),
            pltpu.VMEM((F, D), bf16),
            pltpu.VMEM((16 * D,), bf16),
            pltpu.SemaphoreType.DMA((3,)),
            pltpu.SemaphoreType.DMA((8,)),
            pltpu.SemaphoreType.DMA((S // TP + 1,)),
        ] + [pltpu.VMEM((CK // 2, TQ), u32)] * RING + [pltpu.VMEM((DH, 8, TQ), f32)] * HG,
        compiler_params=pltpu.CompilerParams(vmem_limit_bytes=120 * 1024 * 1024),
    )(A_x.reshape(S, D), A_wqkv, B_w_r, A_wo, B_w_gate, B_w_up, B_w_down)
    return out.reshape(B, S, D)
```

```python
import math

import jax
import jax.numpy as jnp
from jax import lax
import jax.experimental.pallas as pl
import jax.experimental.pallas.tpu as pltpu

f32, bf16, u32, i32 = jnp.float32, jnp.bfloat16, jnp.uint32, jnp.int32

H = 32
DH = 16
HG = 8
TQ = 512
CK = 128
VK = 16
MK = CK - VK
LAG = 4
RING = 8
TP = 2 * CK
EPS = 1e-5
BF16_MAX = 3.3895313892515355e38
F32_TINY = 2.0 ** -126
L_LO, L_HI = 2.0 ** -60, 2.0 ** 60


def _rb(x):
    return x.astype(bf16).astype(f32)


def _mean(x):
    return jnp.sum(x, axis=-1, keepdims=True) * (1.0 / x.shape[-1])


def _layernorm(x):
    xc = x - _mean(x)
    return xc * lax.rsqrt(_mean(xc * xc) + EPS)


def _layernorm_bf16(x):
    mean = _mean(x)
    xc = x - mean
    v = _rb(_rb(_mean(xc * xc)) + EPS)
    den = _rb(v * lax.rsqrt(v))
    inv = pl.reciprocal(den, approx=True)
    inv = inv * (2.0 - den * inv)
    return (x - _rb(mean)) * inv


def _pack(x):
    return pltpu.bitcast(x.astype(bf16), u32)


def _unpack(x):
    return pltpu.bitcast(x, bf16)


def _kernel(x_hbm, wqkv_hbm, wr_hbm, wo_hbm, wg_hbm, wu_hbm, wd_hbm, o_hbm,
            x_ref, xn_ref, wqkv_ref, wt_ref, kp_ref, kv_ref, kb_ref, qp_ref, vp_ref, op_ref,
            l_ref, h_ref, hn_ref, o_ref, wo_ref, wg_ref, wu_ref, wd_ref, wr_ref,
            xsem, wsem, osem, *stage):
    pt_refs = stage[:RING]
    qs_refs = stage[RING:]
    S, D = x_ref.shape
    NQ = S // TQ
    NC = S // CK
    NG = H // HG
    NP = S // TP
    NV = NC * VK
    MR = 2 * MK

    B0, B1 = 1, 5
    x_cuts = (0, NV + B0 * MR, NV + B1 * MR, S)

    def x_copy(n):
        rows = pl.ds(x_cuts[n], x_cuts[n + 1] - x_cuts[n])
        return pltpu.make_async_copy(x_hbm.at[rows, :], x_ref.at[rows, :], xsem.at[n])

    def w_copy(n):
        if n < 3:
            cols = pl.ds(n * D, D)
            return pltpu.make_async_copy(wqkv_hbm.at[:, cols], wqkv_ref.at[:, cols], wsem.at[n])
        src, dst = ((wo_hbm, wo_ref), (wg_hbm, wg_ref), (wu_hbm, wu_ref), (wd_hbm, wd_ref),
                    (wr_hbm, wr_ref.at[pl.ds(0, D)]))[n - 3]
        return pltpu.make_async_copy(src, dst, wsem.at[n])

    x_copy(0).start()
    w_copy(1).start()
    x_copy(1).start()
    x_copy(2).start()
    w_copy(0).start()
    w_copy(2).start()

    def bcast_keys(jds):
        for jd in jds:
            col = jnp.broadcast_to(kv_ref[:, :, jd:jd + 1], kv_ref.shape)
            kb_ref[jd] = _unpack(col).astype(f32)

    def ln_block(b):
        xn = _layernorm(x_ref[NV + b * MR:NV + (b + 1) * MR, :].astype(f32))
        for cc in range(2):
            r0 = (2 * b + cc) * (CK // 2) + VK // 2
            xn_ref[r0:r0 + MK // 2, :] = _pack(xn[cc * MK:(cc + 1) * MK])

    def k_proj(b):
        xu = jnp.concatenate(
            [xn_ref[(2 * b + cc) * (CK // 2) + VK // 2:(2 * b + cc + 1) * (CK // 2), :]
             for cc in range(2)], axis=0)
        k = jnp.dot(_unpack(xu), wqkv_ref[:, D:2 * D], preferred_element_type=f32)
        for g in range(NG):
            kp_ref[g, b * MK:(b + 1) * MK, :] = _pack(k[:, g * 128:(g + 1) * 128])

    early = 4
    jds = [j * DH + d for d in range(early) for j in range(HG)]

    x_copy(0).wait()
    xn0 = _layernorm(x_ref[0:NV, :].astype(f32))
    for c in range(NC):
        xn_ref[c * (CK // 2):c * (CK // 2) + VK // 2, :] = _pack(xn0[c * VK:(c + 1) * VK])
    for b in range(B0):
        ln_block(b)
    w_copy(1).wait()
    kv = jnp.dot(xn0.astype(bf16), wqkv_ref[:, D:2 * D], preferred_element_type=f32)
    for g in range(NG):
        kv_ref[g] = _pack(kv[:, g * 128:(g + 1) * 128])
    bcast_keys(jds[:8])
    x_copy(1).wait()
    for b in range(B0, B1):
        ln_block(b)
    bcast_keys(jds[8:23])
    for b in range(B1 - 1):
        k_proj(b)
    x_copy(2).wait()
    w_copy(0).wait()
    w_copy(2).wait()
    for n in range(3, 8):
        w_copy(n).start()
    for b in range(B1, NP):
        ln_block(b)
    wt_ref[0:D // 2, :] = _pack(wqkv_ref[:, 0:D].astype(f32).T)
    wt_ref[D // 2:D, :] = _pack(wqkv_ref[:, 2 * D:3 * D].astype(f32).T)
    bcast_keys(jds[23:])
    for b in range(B1 - 1, NP):
        k_proj(b)
    qscale = (DH ** -0.5) * math.log2(math.e)
    for b in range(NP):
        bcast_keys([b * DH + d for d in range(early, DH)])
        xp = _unpack(xn_ref[b * (TP // 2):(b + 1) * (TP // 2), :])
        qv = lax.dot_general(_unpack(wt_ref[...]), xp, (((1,), (1,)), ((), ())),
                             preferred_element_type=f32)
        qp_ref[:, b * TP:(b + 1) * TP] = _pack(qv[0:D] * qscale)
        vp_ref[:, b * TP:(b + 1) * TP] = _pack(qv[D:2 * D])

    NI = NQ * NG
    assert NG == 4 and NI & (NI - 1) == 0

    def unit_index(i, j):
        h = (i & (NG - 1)) * HG + j
        return h, pl.multiple_of(h * 8, 8), pl.ds(pl.multiple_of((i >> 2) * TQ, TQ), TQ)

    def stage_q(unit, j, lo, hi):
        _, h8, cols = unit
        qf = _unpack(qp_ref[pl.ds(h8, 8), cols]).astype(f32)
        for d in range(lo, hi):
            qs_refs[j][d] = jnp.broadcast_to(qf[d:d + 1, :], (8, TQ))

    def pv_step(unit, c, row0, acc, inv_l, link=None):
        _, h8, cols = unit
        vt = _unpack(vp_ref[pl.ds(h8, 8), c * CK:(c + 1) * CK])
        d = jnp.dot(vt, _unpack(pt_refs[c % RING][pl.ds(row0, CK // 2), :]),
                    preferred_element_type=f32)
        if acc is None:
            acc = jnp.where(link[0], link[1], d)
        else:
            acc = acc + d
        if c == NC - 1:
            op_ref[pl.ds(h8, 8), cols] = _pack(acc * jnp.concatenate([inv_l, inv_l], axis=0))
        return acc

    def inv_denominator(unit, l8):
        h, _, cols = unit
        l = jnp.sum(l8, axis=0, keepdims=True)
        l_ref[pl.ds(h, 1), cols] = l
        inv = pl.reciprocal(l, approx=True)
        inv = inv * (2.0 - l * inv)
        return jnp.broadcast_to(inv, l8.shape)

    def fast_group(i, carry):
        z1 = lax.shift_right_logical(i, 20)
        row0 = pl.multiple_of(z1 * 8, 8)
        never = lax.broadcasted_iota(i32, (VK, 128), 0) < z1
        never_wide = lax.broadcasted_iota(i32, (DH, TQ), 0) < z1
        g = i & (NG - 1)
        units = {j: unit_index(i, j) for j in range(HG)}
        units[-1] = unit_index((i + NI - 1) & (NI - 1), HG - 1)
        units[HG] = unit_index(jnp.minimum(i + 1, NI - 1), 0)
        dims = [z1 + d0 for d0 in range(0, DH, 4)]
        acc = {-1: carry[0]}
        l8 = {-1: inv_denominator(units[-1], carry[1])}
        pend = [(-1, c) for c in range(NC - LAG, NC)]
        prev = None
        for j in range(HG):
            _, h8, cols = units[j]
            kdims = [d0 + j * DH for d0 in dims]
            qrow = qp_ref[pl.ds(h8, 8), cols]
            z = jnp.zeros_like(qrow)
            w = _unpack(jnp.concatenate([qrow if b == j else z for b in range(HG)], axis=0))
            acc[j] = None
            l8[j] = None
            jn = (j + 1) % HG
            for c in range(NC):
                pt_ref = pt_refs[c % RING]
                base = c * (MK // 2)
                kc = _unpack(jnp.concatenate(
                    [kp_ref[g, base + b * 8:base + (b + 1) * 8, :] for b in range(6, -1, -1)],
                    axis=0))
                p = jnp.exp2(jnp.dot(kc, w, preferred_element_type=f32))
                cl = jnp.sum(p.reshape(MK // 8, 8, TQ), axis=0)
                l8[j] = cl if l8[j] is None else l8[j] + cl
                for b in range(7):
                    pt_ref[(7 - b) * 8:(8 - b) * 8, :] = _pack(p[b * 16:(b + 1) * 16, :])
                pend.append((j, c))
                pj, pc = pend.pop(0)
                link = (never_wide, acc[pj - 1]) if pc == 0 else None
                acc[pj] = pv_step(units[pj], pc, row0, acc[pj], l8[pj], link)

                tie = None
                if c in (7, 9, 11, 13):
                    tie = qs_refs[jn][z1, :, 0:128]
                    tie = jnp.concatenate([tie, tie], axis=0)
                tiles = []
                for t in range(TQ // 128):
                    a = None
                    for d0, kd0 in zip(dims, kdims):
                        kb = kb_ref[pl.ds(kd0, 4), g, c * VK:(c + 1) * VK, :]
                        qd = qs_refs[j][pl.ds(d0, 4), :, t * 128:(t + 1) * 128]
                        pr = kb * jnp.concatenate([qd, qd], axis=1)
                        if a is not None:
                            a = jnp.sum(jnp.concatenate([a[None], pr], axis=0), axis=0)
                            continue
                        a = pr[0]
                        if t == 0 and tie is not None:
                            a = jnp.where(never, tie, a)
                        a = a + pr[1] + pr[2]
                        if prev is not None:
                            a = jnp.where(never, prev, a)
                        a = a + pr[3]
                    prev = a
                    tiles.append(a)
                p = jnp.exp2(jnp.concatenate(tiles, axis=1))
                l8[j] = l8[j] + (p[0:8] + p[8:16])
                pt_ref[0:8, :] = _pack(p)
                if c == NC - 1 and j < HG - 1:
                    l8[j] = inv_denominator(units[j], l8[j])
                if c in (6, 8, 10, 12):
                    stage_q(units[j + 1], jn, (c - 6) * 2, (c - 6) * 2 + 4)
        return acc[HG - 1], l8[HG - 1]

    stage_q(unit_index(0, 0), 0, 0, DH)
    for c in range(NC - LAG, NC):
        pt_refs[c % RING][...] = jnp.zeros((CK // 2, TQ), u32)
    acc, l8 = lax.fori_loop(0, NI, fast_group,
                            (jnp.zeros((DH, TQ), f32), jnp.ones((8, TQ), f32)))
    inv_l = inv_denominator(unit_index(NI - 1, HG - 1), l8)
    for c in range(NC - LAG, NC):
        acc = pv_step(unit_index(NI - 1, HG - 1), c, 0, acc, inv_l)

    l_all = l_ref[...]
    in_window = jnp.logical_and(l_all >= L_LO, l_all <= L_HI)

    @pl.when(jnp.max(jnp.where(in_window, 0.0, 1.0)) > 0.0)
    def _():
        def unit(u, carry):
            h = u % H
            g = h // HG
            j = h % HG
            cols = pl.ds(pl.multiple_of((u // H) * TQ, TQ), TQ)
            h8 = pl.multiple_of(h * 8, 8)
            qrow = qp_ref[pl.ds(h8, 8), cols]
            z = jnp.zeros_like(qrow)
            w = _unpack(jnp.concatenate(
                [jnp.where(j == b, qrow, z) for b in range(HG)], axis=0))

            def scores(c):
                kc = jnp.concatenate(
                    [kv_ref[g, pl.ds(pl.multiple_of(c * 8, 8), 8), :],
                     kp_ref[g, pl.ds(pl.multiple_of(c * (MK // 2), 8), MK // 2), :]], axis=0)
                return jnp.dot(_unpack(kc), w, preferred_element_type=f32)

            def max_body(c, m):
                return jnp.maximum(m, jnp.max(scores(c), axis=0, keepdims=True))

            m = lax.fori_loop(0, NC, max_body, jnp.full((1, TQ), -jnp.inf, f32))

            def sum_body(c, la):
                l, a = la
                p = jnp.exp2(scores(c) - m)
                vt = _unpack(vp_ref[pl.ds(h8, 8), pl.ds(pl.multiple_of(c * CK, CK), CK)])
                a = a + jnp.dot(vt, p.astype(bf16), preferred_element_type=f32)
                return l + jnp.sum(p, axis=0, keepdims=True), a

            l, a = lax.fori_loop(0, NC, sum_body,
                                 (jnp.zeros((1, TQ), f32), jnp.zeros((DH, TQ), f32)))
            op_ref[pl.ds(h8, 8), cols] = _pack(a * (1.0 / l))
            return carry

        lax.fori_loop(0, NQ * H, unit, 0)

    def out_copy(n):
        rows = pl.ds(0, NV) if n == NP else pl.ds(NV + n * MR, MR)
        return pltpu.make_async_copy(o_ref.at[rows, :], o_hbm.at[rows, :], osem.at[n])

    send_after = {7: range(0, 4), 13: range(4, 7), 15: range(7, NP + 1)}

    def token_spans(c):
        return ((0, c * VK, VK), (VK, NV + c * MK, MK))

    for n in range(3, 8):
        w_copy(n).wait()
    wr = jnp.broadcast_to(wr_ref[pl.ds(0, D)].astype(f32).reshape(1, D), (16, D)).astype(bf16)
    wo = wo_ref[...]

    def out_proj(c):
        ot = _unpack(op_ref[:, c * CK:(c + 1) * CK])
        return lax.dot_general(ot, wo, (((0,), (0,)), ((), ())),
                               preferred_element_type=f32)

    def residual_ln(c, attn):
        xb = jnp.concatenate(
            [x_ref[t0:t0 + n, :].astype(f32) for _, t0, n in token_spans(c)], axis=0)
        h = _rb(xb + attn)
        hn = _layernorm_bf16(h).astype(bf16)
        hnf = hn.astype(f32)
        o = h + hnf
        for p0, t0, n in token_spans(c):
            h_ref[t0:t0 + n, :] = h[p0:p0 + n]
            hn_ref[t0:t0 + n, :] = hnf[p0:p0 + n]
            o_ref[t0:t0 + n, :] = o[p0:p0 + n].astype(bf16)
        for n in send_after.get(c, ()):
            out_copy(n).start()
        return hn

    def router(c, hn):
        r = lax.dot_general(wr, hn, (((1,), (1,)), ((), ())), preferred_element_type=f32)
        r = jnp.clip(_rb(r[0:8, :]), -BF16_MAX, BF16_MAX)
        r = jnp.where(jnp.abs(r) < F32_TINY, F32_TINY, r)
        off = lax.broadcasted_iota(i32, r.shape, 1)
        tok = off + jnp.where(off < VK, c * VK, NV + c * MK - VK)
        key = pltpu.bitcast(r, i32) | jnp.where(r < 0, tok, S - 1 - tok)
        return pltpu.bitcast(key, f32)

    attn = out_proj(0)
    hn_prev = None
    keys = []
    for c in range(NC):
        attn_next = out_proj(c + 1) if c + 1 < NC else None
        if hn_prev is not None:
            keys.append(router(c - 1, hn_prev))
        hn_prev = residual_ln(c, attn)
        attn = attn_next
    keys.append(router(NC - 1, hn_prev))

    top, sec = keys[0], jnp.full(keys[0].shape, -jnp.inf, f32)
    for k in keys[1:]:
        sec = jnp.maximum(sec, jnp.minimum(top, k))
        top = jnp.maximum(top, k)
    k1 = jnp.max(top, axis=1, keepdims=True)
    k2 = jnp.max(jnp.where(top == k1, sec, top), axis=1, keepdims=True)

    def decode(k):
        bits = pltpu.bitcast(jnp.broadcast_to(k, (8, 128)), i32)
        low = bits & 0xFFFF
        tok = jnp.where(bits < 0, low, S - 1 - low)
        score = pltpu.bitcast(bits & jnp.int32(-65536), f32)
        return jnp.clip(tok[0, 0], 0, S - 1), score[0:1, 0:1]

    i1, r1 = decode(k1)
    i2, r2 = decode(k2)
    row16 = lax.broadcasted_iota(i32, (16, D), 0)
    first = row16 == 0
    hsel = jnp.where(first, h_ref[pl.ds(i1, 1), :], h_ref[pl.ds(i2, 1), :])
    xsel = jnp.where(first, hn_ref[pl.ds(i1, 1), :], hn_ref[pl.ds(i2, 1), :])
    xs = xsel.astype(bf16)
    gpre = _rb(jnp.dot(xs, wg_ref[...], preferred_element_type=f32))
    gate = _rb(gpre * jax.nn.sigmoid(gpre))
    up = _rb(jnp.dot(xs, wu_ref[...], preferred_element_type=f32))
    y = _rb(jnp.dot((gate * up).astype(bf16), wd_ref[...], preferred_element_type=f32))
    y = _rb(y * _rb(jax.nn.sigmoid(jnp.where(first, r1, r2))))
    osel = hsel + _rb(xsel + y)
    for n in range(NP + 1):
        out_copy(n).wait()
    bases = [pl.multiple_of(lax.shift_right_logical(idx, 4) * 16, 16) for idx in (i1, i2)]
    olds = [o_ref[pl.ds(base, 16), :].astype(f32) for base in bases]
    for base, old in zip(bases, olds):
        t = row16 + base
        new = jnp.where(t == i1, osel[0:1, :], jnp.where(t == i2, osel[1:2, :], old))
        o_ref[pl.ds(base, 16), :] = new.astype(bf16)
    patch = [pltpu.make_async_copy(o_ref.at[pl.ds(base, 16), :], o_hbm.at[pl.ds(base, 16), :],
                                   osem.at[n]) for n, base in enumerate(bases)]
    patch[0].start()

    @pl.when(bases[0] != bases[1])
    def _():
        patch[1].start()
        patch[1].wait()

    patch[0].wait()


@jax.jit
def pallas_sequential_preLN__mha_block__moe_arch_mod__prompt_kernel(
    A_x: jax.Array,
    A_wqkv: jax.Array,
    A_wo: jax.Array,
    B_x: jax.Array,
    B_w_r: jax.Array,
    B_w_gate: jax.Array,
    B_w_up: jax.Array,
    B_w_down: jax.Array,
):
    B, S, D = A_x.shape
    F = B_w_gate.shape[1]
    assert B == 1 and D == H * DH and S == 2048
    hbm = pl.BlockSpec(memory_space=pl.ANY)
    NC = S // CK
    NV = NC * VK
    out = pl.pallas_call(
        _kernel,
        out_shape=jax.ShapeDtypeStruct((S, D), A_x.dtype),
        in_specs=[hbm] * 7,
        out_specs=hbm,
        scratch_shapes=[
            pltpu.VMEM((S, D), bf16),
            pltpu.VMEM((S // 2, D), u32),
            pltpu.VMEM((D, 3 * D), bf16),
            pltpu.VMEM((D, D), u32),
            pltpu.VMEM((H // HG, NC * MK // 2, 128), u32),
            pltpu.VMEM((H // HG, NV // 2, 128), u32),
            pltpu.VMEM((128, H // HG, NV, 128), f32),
            pltpu.VMEM((D // 2, S), u32),
            pltpu.VMEM((D // 2, S), u32),
            pltpu.VMEM((D // 2, S), u32),
            pltpu.VMEM((H, S), f32),
            pltpu.VMEM((S, D), f32),
            pltpu.VMEM((S, D), f32),
            pltpu.VMEM((S, D), bf16),
            pltpu.VMEM((D, D), bf16),
            pltpu.VMEM((D, F), bf16),
            pltpu.VMEM((D, F), bf16),
            pltpu.VMEM((F, D), bf16),
            pltpu.VMEM((16 * D,), bf16),
            pltpu.SemaphoreType.DMA((3,)),
            pltpu.SemaphoreType.DMA((8,)),
            pltpu.SemaphoreType.DMA((S // TP + 1,)),
        ] + [pltpu.VMEM((CK // 2, TQ), u32)] * RING + [pltpu.VMEM((DH, 8, TQ), f32)] * HG,
        compiler_params=pltpu.CompilerParams(vmem_limit_bytes=120 * 1024 * 1024),
    )(A_x.reshape(S, D), A_wqkv, B_w_r, A_wo, B_w_gate, B_w_up, B_w_down)
    return out.reshape(B, S, D)
```
